```python
import jax
import jax.numpy as jnp

def _softmax(x, axis=-1):
    return jax.nn.softmax(x, axis=axis)

def _gelu(x):
    return jax.nn.gelu(x, approximate=True)

def _silu(x):
    return jax.nn.silu(x)

def _sigmoid(x):
    return jax.nn.sigmoid(x)

def _layernorm(x, axis=-1, eps=1e-05):
    m = jnp.mean(x, axis=axis, keepdims=True)
    v = jnp.var(x, axis=axis, keepdims=True)
    return (x - m) / jnp.sqrt(v + eps)

def _scatter_add(tgt, idx, src, axis=0):
    return tgt.at[idx].add(src)

def _segment_sum(src, seg, n):
    return jax.ops.segment_sum(src, seg, n)

class _Rng:

    def __init__(self, key):
        self._k = key

    def _next(self):
        self._k, sub = jax.random.split(self._k)
        return sub

    def normal(self, shape):
        return jax.random.normal(self._next(), shape, dtype=jnp.bfloat16)

    def randint(self, lo, hi, shape):
        return jax.random.randint(self._next(), shape, lo, hi, dtype=jnp.int32)

    def uniform(self, shape, lo=0.0, hi=1.0):
        return jax.random.uniform(self._next(), shape, jnp.bfloat16, lo, hi)

    def permutation(self, n):
        return jax.random.permutation(self._next(), n)
kernel_name = 'adaLN_cond__sliding_block_cached__moe_arch_mod__decode'

def setup_inputs():
    _rng = _Rng(jax.random.key(int.from_bytes(__import__("os").urandom(4), "little")))
    _w = lambda a: (lambda t: t.astype(jnp.bfloat16) if jnp.issubdtype(t.dtype, jnp.floating) else t)(jnp.asarray(a))

    def _A_setup():
        B, Sq, D = (8, 1, 576)
        Hq, Hkv, Sk, Dh = (32, 16, 8192, 128)
        assert Hq % Hkv == 0, (Hq, Hkv)
        return {'x': _w((lambda *s: _rng.normal(s) * 0.05)(B, Sq, D)), 'k_cache': _w((lambda *s: _rng.normal(s) * 0.05)(B, Hkv, Sk, Dh)), 'v_cache': _w((lambda *s: _rng.normal(s) * 0.05)(B, Hkv, Sk, Dh)), 'wq': _w((lambda *s: _rng.normal(s) * 0.05)(D, Hq * Dh) * D ** (-0.5)), 'wo': _w((lambda *s: _rng.normal(s) * 0.05)(Hq * Dh, D) * (Hq * Dh) ** (-0.5))}
    _A_in = _A_setup()

    def _B_setup():
        B, S, D, F, C = (8, 1, 576, 4608, 1)
        return {'x': _w((lambda *s: _rng.normal(s) * 0.05)(B, S, D)), 'w_r': _w((lambda *s: _rng.normal(s) * 0.05)(D)), 'w_gate': _w((lambda *s: _rng.normal(s) * 0.05)(D, F)), 'w_up': _w((lambda *s: _rng.normal(s) * 0.05)(D, F)), 'w_down': _w((lambda *s: _rng.normal(s) * 0.05)(F, D))}
    _B_in = _B_setup()
    return {'A_x': _A_in['x'], 'A_k_cache': _A_in['k_cache'], 'A_v_cache': _A_in['v_cache'], 'A_wq': _A_in['wq'], 'A_wo': _A_in['wo'], 'B_x': _B_in['x'], 'B_w_r': _B_in['w_r'], 'B_w_gate': _B_in['w_gate'], 'B_w_up': _B_in['w_up'], 'B_w_down': _B_in['w_down'], 'c': _w((lambda *s: _rng.normal(s) * 0.05)(8, 576)), 'w_mod': _w((lambda *s: _rng.normal(s) * 0.05)(576, 6 * 576) * 576 ** (-0.5))}

def reference(A_x, A_k_cache, A_v_cache, A_wq, A_wo, B_x, B_w_r, B_w_gate, B_w_up, B_w_down, c, w_mod):

    def _A_ref(x, k_cache, v_cache, wq, wo):
        B, Sq, D = x.shape
        Hq, Dh = (32, 128)
        Hkv, Sk = (k_cache.shape[1], k_cache.shape[2])
        W = min(4096, max(256, Sk // 4))
        rep = Hq // Hkv
        q = (lambda x, *d: x.transpose(*d))((x @ wq).reshape(B, Sq, Hq, Dh), 0, 2, 1, 3)
        k = jnp.repeat(k_cache[:, :, Sk - W:, :], rep, axis=1)
        v = jnp.repeat(v_cache[:, :, Sk - W:, :], rep, axis=1)
        scores = jnp.einsum('bhqd,bhkd->bhqk', q, k) * Dh ** (-0.5)
        p = _softmax(scores, axis=-1)
        o = jnp.einsum('bhqk,bhkd->bhqd', p, v)
        return (lambda x, *d: x.transpose(*d))(o, 0, 2, 1, 3).reshape(B, Sq, Hq * Dh) @ wo

    def _B_ref(x, w_r, w_gate, w_up, w_down):
        B, S, D = x.shape
        C = 1
        r = x @ w_r
        idx = jnp.argsort(-r, axis=-1)[:, :C]
        idx_e = jnp.repeat(idx.reshape(B, C, 1), D, axis=2)
        x_sel = jnp.take_along_axis(x, idx_e, axis=1)
        g = _silu(x_sel @ w_gate)
        u = x_sel @ w_up
        y = g * u @ w_down
        r_sel = _sigmoid(jnp.take_along_axis(r, idx, axis=1))
        y = y * r_sel.reshape(B, C, 1)
        b_off = (jnp.arange(B) * S).reshape(B, 1)
        flat_idx = (idx + b_off).reshape(B * C)
        zero = (x * 0.0).reshape(B * S, D)
        upd = _scatter_add(zero, flat_idx, y.reshape(B * C, D), axis=0)
        return x + upd.reshape(B, S, D)
    x = A_x
    mod = (_silu(c) @ w_mod).reshape(c.shape[0], 6, 1, -1)
    sa, ca, ga, sb, cb, gb = (mod[:, 0].copy(), mod[:, 1].copy(), mod[:, 2].copy(), mod[:, 3].copy(), mod[:, 4].copy(), mod[:, 5].copy())
    h = _layernorm(x, axis=-1) * (1 + ca) + sa
    x = x + ga * _A_ref(h, A_k_cache, A_v_cache, A_wq, A_wo)
    h = _layernorm(x, axis=-1) * (1 + cb) + sb
    x = x + gb * _B_ref(h, B_w_r, B_w_gate, B_w_up, B_w_down)
    return x
```

```python
import functools
import jax
import jax.numpy as jnp
from jax import lax
import jax.experimental.pallas as pl
import jax.experimental.pallas.tpu as pltpu

F32 = jnp.float32
BF16 = jnp.bfloat16
_NT = (((1,), (1,)), ((), ()))


def _layernorm(x, eps=1e-05):
    m = jnp.mean(x, axis=-1, keepdims=True)
    d = x - m
    v = jnp.mean(d * d, axis=-1, keepdims=True)
    return d / jnp.sqrt(v + eps)


def _sigmoid(x):
    return 1.0 / (1.0 + jnp.exp(-x))


def _row_chunks(n, step):
    return [(s, min(step, n - s)) for s in range(0, n, step)]


def make(nslot=3, wchunk=128):
    def fn(A_x, A_k_cache, A_v_cache, A_wq, A_wo, B_x, B_w_r, B_w_gate, B_w_up, B_w_down, c, w_mod):
        B, Sq, D = A_x.shape
        _, Hkv, Sk, Dh = A_k_cache.shape
        Hq = A_wq.shape[1] // Dh
        rep = Hq // Hkv
        F = B_w_gate.shape[1]
        W = min(4096, max(256, Sk // 4))
        assert Sq == 1 and rep == 2 and B == 8
        scale = Dh ** (-0.5)
        chunks = _row_chunks(D, wchunk)
        nch = len(chunks)

        def kernel(x_hbm, k_hbm, v_hbm, wq_hbm, wot_hbm, wr_hbm, wg_hbm, wu_hbm, wdt_hbm, c_hbm, wmod_hbm,
                   o_ref,
                   x_v, c_v, wr_v, wmod_v, wq_v, wot_v, wg_v, wu_v, wdt_v, kbuf, vbuf, q_scr, a_scr,
                   sem_s, sem_w, sem_k, sem_v):
            cp_x = pltpu.make_async_copy(x_hbm, x_v, sem_s.at[0])
            cp_c = pltpu.make_async_copy(c_hbm, c_v, sem_s.at[1])
            cp_r = pltpu.make_async_copy(wr_hbm, wr_v, sem_s.at[2])

            def w_copies(src, dst, i):
                return [pltpu.make_async_copy(src.at[pl.ds(s, n)], dst.at[pl.ds(s, n)], sem_w.at[i, j])
                        for j, (s, n) in enumerate(chunks)]

            cp_mod = w_copies(wmod_hbm, wmod_v, 0)
            cp_wq = w_copies(wq_hbm, wq_v, 1)
            cp_wo = w_copies(wot_hbm, wot_v, 2)
            cp_wg = w_copies(wg_hbm, wg_v, 3)
            cp_wu = w_copies(wu_hbm, wu_v, 4)
            cp_wd = w_copies(wdt_hbm, wdt_v, 5)

            def kv_copy(src, buf, sem, h, slot, b):
                return pltpu.make_async_copy(src.at[b, h, pl.ds(Sk - W, W), :], buf.at[slot, b], sem.at[slot, b])

            def start_all(cps):
                for j, cp in enumerate(cps):
                    cp.start(priority=j % 2)

            def start_kv(src, buf, sem, h, slot):
                for b in range(B):
                    kv_copy(src, buf, sem, h, slot, b).start(priority=b % 2)

            cp_c.start()
            cp_x.start()
            cp_r.start()
            start_all(cp_mod)
            start_all(cp_wq)
            for s in range(nslot):
                start_kv(k_hbm, kbuf, sem_k, s, s)
                start_kv(v_hbm, vbuf, sem_v, s, s)

            cp_c.wait()
            cf = c_v[...].astype(F32)
            sc = (cf * _sigmoid(cf)).astype(BF16)
            for cp in cp_mod:
                cp.wait()
            mod = jnp.dot(sc, wmod_v[...], preferred_element_type=F32)
            sa, ca, ga, sb, cb, gb = [mod[:, i * D:(i + 1) * D] for i in range(6)]
            cp_x.wait()
            x0 = x_v[...].astype(F32)
            h1 = (_layernorm(x0) * (1.0 + ca) + sa).astype(BF16)
            for cp in cp_wq:
                cp.wait()
            q = jnp.dot(h1, wq_v[...], preferred_element_type=F32)
            for h in range(Hkv):
                q2 = jnp.concatenate([q[:, (2 * h) * Dh:(2 * h + 1) * Dh], q[:, (2 * h + 1) * Dh:(2 * h + 2) * Dh]], axis=0)
                q_scr[h] = q2.astype(BF16)

            row_s = lax.broadcasted_iota(jnp.int32, (rep * B, W), 0) % B
            row_o = lax.broadcasted_iota(jnp.int32, (rep * B, Dh), 0) % B
            tail = [cp_wo, cp_wg, cp_wu, cp_wd]

            def head(h, carry):
                slot = h % nslot
                qh = q_scr[h]
                s = None
                for b in range(B):
                    kv_copy(k_hbm, kbuf, sem_k, h, slot, b).wait()
                    sb_ = lax.dot_general(qh, kbuf[slot, b], _NT, preferred_element_type=F32)
                    s = sb_ if s is None else jnp.where(row_s == b, sb_, s)

                @pl.when(h + nslot < Hkv)
                def _():
                    start_kv(k_hbm, kbuf, sem_k, h + nslot, slot)

                for t in range(min(nslot, 2)):
                    @pl.when(h + nslot == Hkv + t)
                    def _():
                        start_all(tail[2 * t])

                s = s * scale
                m = jnp.max(s, axis=-1, keepdims=True)
                p = jnp.exp(s - m)
                l = jnp.sum(p, axis=-1, keepdims=True)
                pb = p.astype(BF16)
                o = None
                for b in range(B):
                    kv_copy(v_hbm, vbuf, sem_v, h, slot, b).wait()
                    ob = jnp.dot(pb, vbuf[slot, b], preferred_element_type=F32)
                    o = ob if o is None else jnp.where(row_o == b, ob, o)

                @pl.when(h + nslot < Hkv)
                def _():
                    start_kv(v_hbm, vbuf, sem_v, h + nslot, slot)

                for t in range(min(nslot, 2)):
                    @pl.when(h + nslot == Hkv + t)
                    def _():
                        start_all(tail[2 * t + 1])

                a_scr[h] = o / l
                return carry

            lax.fori_loop(0, Hkv, head, 0)

            parts = []
            for h in range(Hkv):
                a = a_scr[h]
                parts += [a[0:B], a[B:2 * B]]
            attn = jnp.concatenate(parts, axis=1).astype(BF16)
            for cp in cp_wo:
                cp.wait()
            ao = lax.dot_general(attn, wot_v[...], _NT, preferred_element_type=F32)
            x1 = x0 + ga * ao
            h2f = _layernorm(x1) * (1.0 + cb) + sb
            h2 = h2f.astype(BF16)
            cp_r.wait()
            wr = wr_v[...].astype(F32).reshape(1, D)
            r = jnp.sum(h2.astype(F32) * wr, axis=-1, keepdims=True)
            gate_r = _sigmoid(r)

            def proj(cps, w_v):
                acc = None
                for cp, (s0, n) in zip(cps, chunks):
                    cp.wait()
                    d = jnp.dot(h2[:, s0:s0 + n], w_v[pl.ds(s0, n), :], preferred_element_type=F32)
                    acc = d if acc is None else acc + d
                return acc

            g = proj(cp_wg, wg_v)
            g = g * _sigmoid(g)
            u = proj(cp_wu, wu_v)
            act = (g * u).astype(BF16)
            for cp, (s0, n) in zip(cp_wd, chunks):
                cp.wait()
                y = lax.dot_general(act, wdt_v[pl.ds(s0, n), :], _NT, preferred_element_type=F32)
                hh = h2f[:, s0:s0 + n]
                upd = hh * 0.0 + y * gate_r
                o_ref[:, s0:s0 + n] = (x1[:, s0:s0 + n] + gb[:, s0:s0 + n] * (hh + upd)).astype(o_ref.dtype)

        any_spec = pl.BlockSpec(memory_space=pl.ANY)
        out = pl.pallas_call(
            kernel,
            out_shape=jax.ShapeDtypeStruct((B, D), A_x.dtype),
            in_specs=[any_spec] * 11,
            out_specs=pl.BlockSpec(memory_space=pltpu.VMEM),
            scratch_shapes=[
                pltpu.VMEM((B, D), BF16), pltpu.VMEM((B, D), BF16), pltpu.VMEM((D,), BF16),
                pltpu.VMEM((D, 6 * D), BF16), pltpu.VMEM((D, Hq * Dh), BF16), pltpu.VMEM((D, Hq * Dh), BF16),
                pltpu.VMEM((D, F), BF16), pltpu.VMEM((D, F), BF16), pltpu.VMEM((D, F), BF16),
                pltpu.VMEM((nslot, B, W, Dh), BF16), pltpu.VMEM((nslot, B, W, Dh), BF16),
                pltpu.VMEM((Hkv, rep * B, Dh), BF16), pltpu.VMEM((Hkv, rep * B, Dh), F32),
                pltpu.SemaphoreType.DMA((3,)), pltpu.SemaphoreType.DMA((6, nch)),
                pltpu.SemaphoreType.DMA((nslot, B)), pltpu.SemaphoreType.DMA((nslot, B)),
            ],
            compiler_params=pltpu.CompilerParams(vmem_limit_bytes=100 * 1024 * 1024),
            name="adaln_attn_moe_decode",
        )(A_x.reshape(B, D), A_k_cache, A_v_cache, A_wq, A_wo.T, B_w_r, B_w_gate, B_w_up, B_w_down.T, c, w_mod)
        return out.reshape(B, Sq, D)
    return fn


_impl = make(nslot=3)


@jax.jit
def pallas_adaLN_cond__sliding_block_cached__moe_arch_mod__decode_kernel(
    A_x: jax.Array,
    A_k_cache: jax.Array,
    A_v_cache: jax.Array,
    A_wq: jax.Array,
    A_wo: jax.Array,
    B_x: jax.Array,
    B_w_r: jax.Array,
    B_w_gate: jax.Array,
    B_w_up: jax.Array,
    B_w_down: jax.Array,
    c: jax.Array,
    w_mod: jax.Array,
):
    return _impl(A_x, A_k_cache, A_v_cache, A_wq, A_wo, B_x, B_w_r, B_w_gate, B_w_up, B_w_down, c, w_mod)
```

```python
import contextlib
import jax
import jax.numpy as jnp
from jax import lax
import jax.experimental.pallas as pl
import jax.experimental.pallas.tpu as pltpu

F32 = jnp.float32
BF16 = jnp.bfloat16
_NT = (((1,), (1,)), ((), ()))


def _layernorm(x, eps=1e-05):
    m = jnp.mean(x, axis=-1, keepdims=True)
    d = x - m
    v = jnp.mean(d * d, axis=-1, keepdims=True)
    return d / jnp.sqrt(v + eps)


def _sigmoid(x):
    return 1.0 / (1.0 + jnp.exp(-x))


def make(nslot=2, dchunks=(128, 128, 128, 128, 64), scopes=False, nosem=False, nobounds=False,
         tail_prio=1, kprio=0, vprio=0, tail_at=None, kvsplit=1):
    S = (lambda n: jax.named_scope(n)) if scopes else (lambda n: contextlib.nullcontext())

    def fn(A_x, A_k_cache, A_v_cache, A_wq, A_wo, B_x, B_w_r, B_w_gate, B_w_up, B_w_down, c, w_mod):
        B, Sq, D = A_x.shape
        _, Hkv, Sk, Dh = A_k_cache.shape
        Hq = A_wq.shape[1] // Dh
        rep = Hq // Hkv
        F = B_w_gate.shape[1]
        W = min(4096, max(256, Sk // 4))
        assert Sq == 1 and rep == 2 and B == 8 and sum(dchunks) == D
        scale = Dh ** (-0.5)
        dch = []
        s0 = 0
        for n in dchunks:
            dch.append((s0, n))
            s0 += n
        NS_FIXED = 5
        nsem = NS_FIXED + len(dch) + 2 * nslot * kvsplit
        bs = B // kvsplit

        def kernel(x_hbm, k_hbm, v_hbm, wq_hbm, wot_hbm, wr_hbm, wg_hbm, wu_hbm, wdt_hbm, c_hbm, wmod_hbm,
                   o_ref,
                   x_v, c_v, wr_v, wmod_v, wq_v, wot_v, wg_v, wu_v, wdt_v, kbuf, vbuf, q_scr, a_scr, sem):
            mk = pltpu.make_async_copy
            cp_head = [mk(wmod_hbm.at[:, pl.ds(0, 2 * D)], wmod_v.at[:, pl.ds(0, 2 * D)], sem.at[0]),
                       mk(c_hbm, c_v, sem.at[0]), mk(x_hbm, x_v, sem.at[0])]
            cp_wq = mk(wq_hbm, wq_v, sem.at[1])
            cp_mid = [mk(wmod_hbm.at[:, pl.ds(2 * D, 4 * D)], wmod_v.at[:, pl.ds(2 * D, 4 * D)], sem.at[2]),
                      mk(wr_hbm, wr_v, sem.at[2]), mk(wot_hbm, wot_v, sem.at[2])]
            cp_wg = mk(wg_hbm, wg_v, sem.at[3])
            cp_wu = mk(wu_hbm, wu_v, sem.at[4])
            cp_wd = [mk(wdt_hbm.at[pl.ds(s, n)], wdt_v.at[pl.ds(s, n)], sem.at[NS_FIXED + j])
                     for j, (s, n) in enumerate(dch)]
            kv0 = NS_FIXED + len(dch)

            def kv_copy(which, h, slot, j):
                src, buf = ((k_hbm, kbuf), (v_hbm, vbuf))[which]
                return mk(src.at[pl.ds(j * bs, bs), h, pl.ds(Sk - W, W), :], buf.at[slot, pl.ds(j * bs, bs)],
                          sem.at[kv0 + (which * nslot + slot) * kvsplit + j])

            def start_kv(which, h, slot):
                for j in range(kvsplit):
                    kv_copy(which, h, slot, j).start(priority=(kprio, vprio)[which])

            def start_tail():
                for cp in cp_mid + [cp_wg, cp_wu] + cp_wd:
                    cp.start(priority=tail_prio)

            with S("issue"):
                for cp in cp_head:
                    cp.start()
                cp_wq.start()
                for s in range(nslot):
                    start_kv(0, s, s)
                    start_kv(1, s, s)
                if tail_at is None:
                    start_tail()

            with S("w_head"):
                for cp in cp_head:
                    cp.wait()
            cf = c_v[...].astype(F32)
            sc = (cf * _sigmoid(cf)).astype(BF16)
            mod_a = jnp.dot(sc, wmod_v[:, 0:2 * D], preferred_element_type=F32)
            sa, ca = mod_a[:, 0:D], mod_a[:, D:2 * D]
            x0 = x_v[...].astype(F32)
            h1 = (_layernorm(x0) * (1.0 + ca) + sa).astype(BF16)
            with S("w_wq"):
                cp_wq.wait()
            q = jnp.dot(h1, wq_v[...], preferred_element_type=F32)
            for h in range(Hkv):
                q2 = jnp.concatenate([q[:, (2 * h) * Dh:(2 * h + 1) * Dh], q[:, (2 * h + 1) * Dh:(2 * h + 2) * Dh]], axis=0)
                q_scr[h] = q2.astype(BF16)

            row_s = lax.broadcasted_iota(jnp.int32, (rep * B, W), 0) % B
            row_o = lax.broadcasted_iota(jnp.int32, (rep * B, Dh), 0) % B

            def head(h, carry):
                slot = h % nslot
                qh = q_scr[h]
                s = None
                for b in range(B):
                    if b % bs == 0:
                        with S("wk%d" % b):
                            kv_copy(0, h, slot, b // bs).wait()
                    sb_ = lax.dot_general(qh, kbuf[slot, b], _NT, preferred_element_type=F32)
                    s = sb_ if s is None else jnp.where(row_s == b, sb_, s)

                @pl.when(h + nslot < Hkv)
                def _():
                    start_kv(0, h + nslot, slot)

                s = s * scale
                m = jnp.max(s, axis=-1, keepdims=True)
                p = jnp.exp(s - m)
                l = jnp.sum(p, axis=-1, keepdims=True)
                pb = p.astype(BF16)
                o = None
                for b in range(B):
                    if b % bs == 0:
                        with S("wv%d" % b):
                            kv_copy(1, h, slot, b // bs).wait()
                    ob = jnp.dot(pb, vbuf[slot, b], preferred_element_type=F32)
                    o = ob if o is None else jnp.where(row_o == b, ob, o)

                @pl.when(h + nslot < Hkv)
                def _():
                    start_kv(1, h + nslot, slot)

                if tail_at is not None:
                    @pl.when(h == tail_at)
                    def _():
                        start_tail()

                a_scr[h] = o / l
                return carry

            lax.fori_loop(0, Hkv, head, 0)

            parts = []
            for h in range(Hkv):
                a = a_scr[h]
                parts += [a[0:B], a[B:2 * B]]
            attn = jnp.concatenate(parts, axis=1).astype(BF16)
            with S("w_mid"):
                for cp in cp_mid:
                    cp.wait()
            mod_b = jnp.dot(sc, wmod_v[:, 2 * D:6 * D], preferred_element_type=F32)
            ga, sb, cb, gb = [mod_b[:, i * D:(i + 1) * D] for i in range(4)]
            ao = lax.dot_general(attn, wot_v[...], _NT, preferred_element_type=F32)
            x1 = x0 + ga * ao
            h2f = _layernorm(x1) * (1.0 + cb) + sb
            h2 = h2f.astype(BF16)
            wr = wr_v[...].astype(F32).reshape(1, D)
            r = jnp.sum(h2.astype(F32) * wr, axis=-1, keepdims=True)
            gate_r = _sigmoid(r)
            with S("w_g"):
                cp_wg.wait()
            g = jnp.dot(h2, wg_v[...], preferred_element_type=F32)
            g = g * _sigmoid(g)
            with S("w_u"):
                cp_wu.wait()
            u = jnp.dot(h2, wu_v[...], preferred_element_type=F32)
            act = (g * u).astype(BF16)
            for cp, (s0, n) in zip(cp_wd, dch):
                with S("w_d%d" % s0):
                    cp.wait()
                y = lax.dot_general(act, wdt_v[pl.ds(s0, n), :], _NT, preferred_element_type=F32)
                hh = h2f[:, s0:s0 + n]
                upd = hh * 0.0 + y * gate_r
                o_ref[:, s0:s0 + n] = (x1[:, s0:s0 + n] + gb[:, s0:s0 + n] * (hh + upd)).astype(o_ref.dtype)

        any_spec = pl.BlockSpec(memory_space=pl.ANY)
        out = pl.pallas_call(
            kernel,
            out_shape=jax.ShapeDtypeStruct((B, D), A_x.dtype),
            in_specs=[any_spec] * 11,
            out_specs=pl.BlockSpec(memory_space=pltpu.VMEM),
            scratch_shapes=[
                pltpu.VMEM((B, D), BF16), pltpu.VMEM((B, D), BF16), pltpu.VMEM((D,), BF16),
                pltpu.VMEM((D, 6 * D), BF16), pltpu.VMEM((D, Hq * Dh), BF16), pltpu.VMEM((D, Hq * Dh), BF16),
                pltpu.VMEM((D, F), BF16), pltpu.VMEM((D, F), BF16), pltpu.VMEM((D, F), BF16),
                pltpu.VMEM((nslot, B, W, Dh), BF16), pltpu.VMEM((nslot, B, W, Dh), BF16),
                pltpu.VMEM((Hkv, rep * B, Dh), BF16), pltpu.VMEM((Hkv, rep * B, Dh), F32),
                pltpu.SemaphoreType.DMA((nsem,)),
            ],
            compiler_params=pltpu.CompilerParams(vmem_limit_bytes=100 * 1024 * 1024,
                                                 disable_semaphore_checks=nosem, disable_bounds_checks=nobounds),
            name="adaln_attn_moe_decode",
        )(A_x.reshape(B, D), A_k_cache, A_v_cache, A_wq, A_wo.T, B_w_r, B_w_gate, B_w_up, B_w_down.T, c, w_mod)
        return out.reshape(B, Sq, D)
    return fn


_impl = make()


@jax.jit
def pallas_adaLN_cond__sliding_block_cached__moe_arch_mod__decode_kernel(
    A_x: jax.Array,
    A_k_cache: jax.Array,
    A_v_cache: jax.Array,
    A_wq: jax.Array,
    A_wo: jax.Array,
    B_x: jax.Array,
    B_w_r: jax.Array,
    B_w_gate: jax.Array,
    B_w_up: jax.Array,
    B_w_down: jax.Array,
    c: jax.Array,
    w_mod: jax.Array,
):
    return _impl(A_x, A_k_cache, A_v_cache, A_wq, A_wo, B_x, B_w_r, B_w_gate, B_w_up, B_w_down, c, w_mod)
```

```python
import contextlib
import jax
import jax.numpy as jnp
from jax import lax
import jax.experimental.pallas as pl
import jax.experimental.pallas.tpu as pltpu

F32 = jnp.float32
BF16 = jnp.bfloat16
_NT = (((1,), (1,)), ((), ()))


def _layernorm(x, eps=1e-05):
    m = jnp.mean(x, axis=-1, keepdims=True)
    d = x - m
    v = jnp.mean(d * d, axis=-1, keepdims=True)
    return d / jnp.sqrt(v + eps)


def _sigmoid(x):
    return 1.0 / (1.0 + jnp.exp(-x))


def make(ch=128, ks=512, scopes=False, nosem=False, nobounds=False, sched=None):
    S = (lambda n: jax.named_scope(n)) if scopes else (lambda n: contextlib.nullcontext())
    sch = dict(pv=0, wo=53, wo_step=3, u_step=3, g=125, g_step=3)
    sch.update(sched or {})

    def fn(A_x, A_k_cache, A_v_cache, A_wq, A_wo, B_x, B_w_r, B_w_gate, B_w_up, B_w_down, c, w_mod):
        B, Sq, D = A_x.shape
        _, Hkv, Sk, Dh = A_k_cache.shape
        Hq = A_wq.shape[1] // Dh
        rep = Hq // Hkv
        F = B_w_gate.shape[1]
        W = min(4096, max(256, Sk // 4))
        assert Sq == 1 and rep == 2 and B == 8
        scale = Dh ** (-0.5)
        M = rep * B
        sizes = [ch] * (W // ch) if isinstance(ch, int) else list(ch)
        assert sum(sizes) == W
        offs = [sum(sizes[:i]) for i in range(len(sizes))]
        nev = len(sizes)
        nsl = W // ks
        NV = 4
        HALF = D // 2
        S_MOD, S_WQ, S_WO, S_WG, S_WU, S_WD = 0, 1, 2, 3, 4, 5
        dpieces = [(0, 128), (288, 96), (128, 128), (256, 32), (384, 128), (512, 64)]
        S_K = S_WD + len(dpieces)
        S_V = S_K + 4
        nsem = S_V + NV

        def kernel(x_hbm, k_hbm, v_hbm, wq_hbm, wot_hbm, wr_hbm, wg_hbm, wu_hbm, wdt_hbm, c_hbm, wmod_hbm,
                   o_ref,
                   x_v, c_v, wr_v, wmod_v, wq_v, wot_v, wg_v, wu_v, wdt_v, kbuf, vbuf,
                   q_scr, a_scr, s_scr, p_scr, l_scr, h_scr, mod_scr, sem):
            mk = pltpu.make_async_copy

            def wait_all(dst, i):
                mk(dst, dst, sem.at[i]).wait()

            def stripe(src, dst, r0, part, nparts, i, prio):
                n = src.shape[1] // nparts
                idx = (pl.ds(r0, 8), pl.ds(part * n, n))
                mk(src.at[idx], dst.at[idx], sem.at[i]).start(priority=prio)

            def kv_event(h, b, j):
                rows, n = offs[j], sizes[j]
                mk(k_hbm.at[b, h, pl.ds(Sk - W + rows, n), :], kbuf.at[h % 2, b, pl.ds(rows, n)],
                   sem.at[S_K + (h % 2) * 2 + b // (B // 2)]).start(priority=0)
                mk(v_hbm.at[b, h, pl.ds(Sk - W + rows, n), :], vbuf.at[h % NV, b, pl.ds(rows, n)],
                   sem.at[S_V + h % NV]).start(priority=1)

            def mod_events(i, carry):
                r0 = pl.multiple_of(i * 8, 8)
                stripe(wmod_hbm, wmod_v, r0, 0, 1, S_MOD, 0)
                stripe(wmod_hbm, wmod_v, r0 + HALF, 0, 1, S_MOD, 1)
                return carry

            def wq_events(i, carry):
                r0 = pl.multiple_of(i * 8, 8)
                for part in range(2):
                    stripe(wq_hbm, wq_v, r0, part, 2, S_WQ, 0)
                    stripe(wq_hbm, wq_v, r0 + HALF, part, 2, S_WQ, 1)
                return carry

            small = [mk(c_hbm, c_v, sem.at[S_MOD]), mk(x_hbm, x_v, sem.at[S_MOD]), mk(wr_hbm, wr_v, sem.at[S_MOD])]
            with S("head"):
                lax.fori_loop(0, HALF // 8, mod_events, 0)
                for cp in small:
                    cp.start()
                lax.fori_loop(0, HALF // 8, wq_events, 0)
            s_scr[...] = jnp.zeros_like(s_scr)

            def do_mod():
                for cp in small:
                    cp.wait()
                wait_all(wmod_v, S_MOD)
                cf = c_v[...].astype(F32)
                sc = (cf * _sigmoid(cf)).astype(BF16)
                mod_a = jnp.dot(sc, wmod_v[:, 0:2 * D], preferred_element_type=F32)
                sa, ca = mod_a[:, 0:D], mod_a[:, D:2 * D]
                h_scr[...] = _layernorm(x_v[...].astype(F32)) * (1.0 + ca) + sa

            def do_mod_b(i):
                cf = c_v[...].astype(F32)
                sc = (cf * _sigmoid(cf)).astype(BF16)
                mb = jnp.dot(sc, wmod_v[:, (2 + 2 * i) * D:(4 + 2 * i) * D], preferred_element_type=F32)
                mod_scr[2 * i] = mb[:, 0:D]
                mod_scr[2 * i + 1] = mb[:, D:2 * D]

            NQ = 4

            def do_q(i):
                if i == 0:
                    wait_all(wq_v, S_WQ)
                nh = Hkv // NQ
                q = jnp.dot(h_scr[...].astype(BF16), wq_v[:, i * nh * rep * Dh:(i + 1) * nh * rep * Dh],
                            preferred_element_type=F32)
                for t in range(nh):
                    q2 = jnp.concatenate([q[:, (rep * t + r) * Dh:(rep * t + r + 1) * Dh] for r in range(rep)], axis=0)
                    q_scr[i * nh + t] = q2.astype(BF16)

            def first_step(b, carry):
                for j in range(nev // 2):
                    kv_event(0, b, j)
                pre = {3: do_mod, 4: lambda: do_q(0), 5: lambda: do_q(2), 6: lambda: do_mod_b(0)}
                for bb, f in pre.items():
                    pl.when(b == bb)(f)
                for j in range(nev // 2, nev):
                    kv_event(0, b, j)
                post = {4: lambda: do_q(1), 5: lambda: do_q(3), 6: lambda: do_mod_b(1)}
                for bb, f in post.items():
                    pl.when(b == bb)(f)
                return carry

            with S("first"):
                lax.fori_loop(0, B, first_step, 0)

            row_s = lax.broadcasted_iota(jnp.int32, (M, ks), 0) % B
            row_o = lax.broadcasted_iota(jnp.int32, (M, Dh), 0) % B

            def qk_slice(h, b, g):
                cols = pl.ds(g * ks, ks)
                sn = lax.dot_general(q_scr[h], kbuf[h % 2, b, cols], _NT, preferred_element_type=F32)
                s_scr[:, cols] = jnp.where(row_s == b, sn, s_scr[:, cols])

            def pv_slice(h, b, g):
                cols = pl.ds(g * ks, ks)
                return jnp.dot(p_scr[:, cols], vbuf[h % NV, b, cols], preferred_element_type=F32)

            def softmax():
                s = s_scr[...] * scale
                m = jnp.max(s, axis=-1, keepdims=True)
                p = jnp.exp(s - m)
                l_scr[...] = jnp.broadcast_to(jnp.sum(p, axis=-1, keepdims=True), (M, Dh))
                p_scr[...] = p.astype(BF16)

            def phase(h, event, n_events, do_pv):
                if do_pv:
                    wait_all(vbuf.at[(h - 1) % NV], S_V + (h - 1) % NV)

                def step(b, o_acc):
                    @pl.when(b % (B // 2) == 0)
                    def _():
                        wait_all(kbuf.at[h % 2, pl.ds(b, B // 2)], S_K + (h % 2) * 2 + b // (B // 2))
                    o = None
                    e = 0
                    for g in range(2 * nsl):
                        e_end = (g + 1) * n_events // (2 * nsl)
                        for j in range(e, e_end):
                            event(b, j)
                        e = e_end
                        if g % 2 == 0:
                            qk_slice(h, b, g // 2)
                        elif do_pv:
                            d = pv_slice(h - 1, b, g // 2)
                            o = d if o is None else o + d
                    return jnp.where(row_o == b, o, o_acc) if do_pv else o_acc

                o_acc = lax.fori_loop(0, B, step, jnp.zeros((M, Dh), F32))
                if do_pv:
                    a_scr[h - 1] = o_acc / l_scr[...]
                softmax()

            with S("ph0"):
                phase(0, lambda b, j: kv_event(1, b, j), nev, False)

            def main(h, carry):
                with S("ph"):
                    phase(h, lambda b, j: kv_event(h + 1, b, j), nev, True)
                return carry

            lax.fori_loop(1, Hkv - 1, main, 0)

            def wo_wu_event(b, j):
                r0 = pl.multiple_of(b * 64 + (j // 2) * 8, 8)
                stripe(wu_hbm, wu_v, r0, j % 2, 2, S_WU, 0)
                stripe(wot_hbm, wot_v, r0, j % 2, 2, S_WO, 1)

            with S("phlast"):
                phase(Hkv - 1, wo_wu_event, 16, True)

            events = []
            for r0 in range(B * 64, D, 8):
                for part in range(2):
                    events.append(lambda r0=r0, part=part: (stripe(wu_hbm, wu_v, r0, part, 2, S_WU, 0),
                                                            stripe(wot_hbm, wot_v, r0, part, 2, S_WO, 1)))
            for r0 in range(0, HALF, 8):
                for part in range(2):
                    events.append(lambda r0=r0, part=part: (stripe(wg_hbm, wg_v, r0, part, 2, S_WG, 0),
                                                            stripe(wg_hbm, wg_v, r0 + HALF, part, 2, S_WG, 1)))

            def dsem(r):
                return S_WD + [i for i, (s0, n) in enumerate(dpieces) if s0 <= r < s0 + n][0]

            for r0 in range(0, HALF, 8):
                for part in range(2):
                    events.append(lambda r0=r0, part=part: (stripe(wdt_hbm, wdt_v, r0, part, 2, dsem(r0), 0),
                                                            stripe(wdt_hbm, wdt_v, r0 + HALF, part, 2, dsem(r0 + HALF), 1)))
            pos = [0]

            def advance_to(e):
                e = min(e, len(events))
                while pos[0] < e:
                    events[pos[0]]()
                    pos[0] += 1

            def advance(n):
                advance_to(pos[0] + n)

            h = Hkv - 1
            wait_all(vbuf.at[h % NV], S_V + h % NV)
            o_acc = jnp.zeros((M, Dh), F32)
            with S("pvlast"):
                for b in range(B):
                    o = None
                    for g in range(nsl):
                        advance(1)
                        d = pv_slice(h, b, g)
                        o = d if o is None else o + d
                    o_acc = jnp.where(row_o == b, o, o_acc)
                a_scr[h] = o_acc / l_scr[...]

            advance_to(sch["wo"])
            with S("w_wo"):
                wait_all(wot_v, S_WO)
            ao = None
            NO = 8
            for i in range(NO):
                nh = Hkv // NO
                parts = []
                for t in range(i * nh, (i + 1) * nh):
                    a = a_scr[t]
                    parts += [a[r * B:(r + 1) * B] for r in range(rep)]
                attn = jnp.concatenate(parts, axis=1).astype(BF16)
                n = nh * rep * Dh
                d = lax.dot_general(attn, wot_v[:, i * n:(i + 1) * n], _NT, preferred_element_type=F32)
                ao = d if ao is None else ao + d
                advance(sch["wo_step"])
            x1 = x_v[...].astype(F32) + mod_scr[0] * ao
            h2f = _layernorm(x1) * (1.0 + mod_scr[2]) + mod_scr[1]
            h2 = h2f.astype(BF16)
            wr = wr_v[...].astype(F32).reshape(1, D)
            gate_r = _sigmoid(jnp.sum(h2.astype(F32) * wr, axis=-1, keepdims=True))
            gb = mod_scr[3]
            advance(1)

            NF = 6
            nf = F // NF
            with S("w_u"):
                wait_all(wu_v, S_WU)
            us = []
            for i in range(NF):
                us.append(jnp.dot(h2, wu_v[:, i * nf:(i + 1) * nf], preferred_element_type=F32))
                advance(sch["u_step"])
            advance_to(sch["g"])
            with S("w_g"):
                wait_all(wg_v, S_WG)
            acts = []
            for i in range(NF):
                g = jnp.dot(h2, wg_v[:, i * nf:(i + 1) * nf], preferred_element_type=F32)
                acts.append((g * _sigmoid(g) * us[i]).astype(BF16))
                advance(sch["g_step"])
            act = jnp.concatenate(acts, axis=1)
            ready = [88 + 32, 88 + 24 + 37, 88 + 64 + 5, 999, 999, 999]
            for i, (s0, n) in enumerate(dpieces):
                advance_to(ready[i])
                with S("w_d%d" % s0):
                    wait_all(wdt_v.at[pl.ds(s0, n)], S_WD + i)
                y = None
                for t in range(2):
                    cols = slice(t * (F // 2), (t + 1) * (F // 2))
                    d = lax.dot_general(act[:, cols], wdt_v[pl.ds(s0, n), cols], _NT, preferred_element_type=F32)
                    y = d if y is None else y + d
                    advance(3)
                hh = h2f[:, s0:s0 + n]
                upd = hh * 0.0 + y * gate_r
                o_ref[:, s0:s0 + n] = (x1[:, s0:s0 + n] + gb[:, s0:s0 + n] * (hh + upd)).astype(o_ref.dtype)
            assert pos[0] == len(events)

        any_spec = pl.BlockSpec(memory_space=pl.ANY)
        out = pl.pallas_call(
            kernel,
            out_shape=jax.ShapeDtypeStruct((B, D), A_x.dtype),
            in_specs=[any_spec] * 11,
            out_specs=pl.BlockSpec(memory_space=pltpu.VMEM),
            scratch_shapes=[
                pltpu.VMEM((B, D), BF16), pltpu.VMEM((B, D), BF16), pltpu.VMEM((D,), BF16),
                pltpu.VMEM((D, 6 * D), BF16), pltpu.VMEM((D, Hq * Dh), BF16), pltpu.VMEM((D, Hq * Dh), BF16),
                pltpu.VMEM((D, F), BF16), pltpu.VMEM((D, F), BF16), pltpu.VMEM((D, F), BF16),
                pltpu.VMEM((2, B, W, Dh), BF16), pltpu.VMEM((NV, B, W, Dh), BF16),
                pltpu.VMEM((Hkv, M, Dh), BF16), pltpu.VMEM((Hkv, M, Dh), F32),
                pltpu.VMEM((M, W), F32), pltpu.VMEM((M, W), BF16), pltpu.VMEM((M, Dh), F32),
                pltpu.VMEM((B, D), F32), pltpu.VMEM((4, B, D), F32),
                pltpu.SemaphoreType.DMA((nsem,)),
            ],
            compiler_params=pltpu.CompilerParams(vmem_limit_bytes=100 * 1024 * 1024,
                                                 disable_semaphore_checks=nosem, disable_bounds_checks=nobounds),
            name="adaln_attn_moe_decode",
        )(A_x.reshape(B, D), A_k_cache, A_v_cache, A_wq, A_wo.T, B_w_r, B_w_gate, B_w_up, B_w_down.T, c, w_mod)
        return out.reshape(B, Sq, D)
    return fn


_impl = make()


@jax.jit
def pallas_adaLN_cond__sliding_block_cached__moe_arch_mod__decode_kernel(
    A_x: jax.Array,
    A_k_cache: jax.Array,
    A_v_cache: jax.Array,
    A_wq: jax.Array,
    A_wo: jax.Array,
    B_x: jax.Array,
    B_w_r: jax.Array,
    B_w_gate: jax.Array,
    B_w_up: jax.Array,
    B_w_down: jax.Array,
    c: jax.Array,
    w_mod: jax.Array,
):
    return _impl(A_x, A_k_cache, A_v_cache, A_wq, A_wo, B_x, B_w_r, B_w_gate, B_w_up, B_w_down, c, w_mod)
```

```python
import contextlib
import jax
import jax.numpy as jnp
from jax import lax
import jax.experimental.pallas as pl
import jax.experimental.pallas.tpu as pltpu

F32 = jnp.float32
BF16 = jnp.bfloat16
_NT = (((1,), (1,)), ((), ()))


def _layernorm(x, eps=1e-05):
    m = jnp.mean(x, axis=-1, keepdims=True)
    d = x - m
    v = jnp.mean(d * d, axis=-1, keepdims=True)
    return d / jnp.sqrt(v + eps)


def _sigmoid(x):
    return 1.0 / (1.0 + jnp.exp(-x))


def make(ch=128, ks=1024, scopes=False, nosem=False, nobounds=False, sched=None, cgroups=(18,), lastw=256, vch=None, scoped=True, unroll0=False, unrolll=False):
    S = (lambda n: jax.named_scope(n)) if scopes else (lambda n: contextlib.nullcontext())
    sch = dict(wo=60, wo_step=3, u_step=2, g=116, g_step=2)
    sch.update(sched or {})

    def fn(A_x, A_k_cache, A_v_cache, A_wq, A_wo, B_x, B_w_r, B_w_gate, B_w_up, B_w_down, c, w_mod):
        B, Sq, D = A_x.shape
        _, Hkv, Sk, Dh = A_k_cache.shape
        Hq = A_wq.shape[1] // Dh
        rep = Hq // Hkv
        F = B_w_gate.shape[1]
        W = min(4096, max(256, Sk // 4))
        assert Sq == 1 and rep == 2 and B == 8 and D == 576
        scale = Dh ** (-0.5)
        M = rep * B
        sizes = [ch] * (W // ch) if isinstance(ch, int) else list(ch)
        assert sum(sizes) == W
        offs = [sum(sizes[:i]) for i in range(len(sizes))]
        vsizes = sizes if vch is None else list(vch)
        assert sum(vsizes) == W and len(vsizes) == len(sizes)
        voffs = [sum(vsizes[:i]) for i in range(len(vsizes))]
        nev = len(sizes)
        nsl = W // ks
        NV = 4
        HALF = D // 2
        S_WO, S_WG, S_WU, S_MOD, S_WQ, S_K, S_V = 0, 1, 2, 3, 4, 5, 9
        nsem = S_V + NV
        S_FREE = 3
        assert sum(cgroups) * lastw == F

        def kernel(x_hbm, k_hbm, v_hbm, wq_hbm, wot_hbm, wr_hbm, wg_hbm, wu_hbm, wdt_hbm, c_hbm, wmod_hbm,
                   o_ref,
                   x_v, c_v, wr_v, wmod_v, wq_v, wot_v, wg_v, wu_v, wdt_v, kbuf, vbuf,
                   q_scr, a_scr, s_scr, p_scr, l_scr, h_scr, mod_scr, sem_last, *maybe_sem):
          mk = pltpu.make_async_copy

          def body(sem):

            def wait_all(dst, i):
                mk(dst, dst, sem.at[i]).wait()

            def stripe(src, dst, r0, part, nparts, i, prio):
                n = src.shape[1] // nparts
                idx = (pl.ds(r0, 8), pl.ds(part * n, n))
                mk(src.at[idx], dst.at[idx], sem.at[i]).start(priority=prio)

            def kv_event(h, b, j):
                rows, n = offs[j], sizes[j]
                mk(k_hbm.at[b, h, pl.ds(Sk - W + rows, n), :], kbuf.at[h % 2, b, pl.ds(rows, n)],
                   sem.at[S_K + (h % 2) * 2 + b // (B // 2)]).start(priority=0)
                rows, n = voffs[j], vsizes[j]
                mk(v_hbm.at[b, h, pl.ds(Sk - W + rows, n), :], vbuf.at[h % NV, b, pl.ds(rows, n)],
                   sem.at[S_V + h % NV]).start(priority=1)

            def prefix(i, carry):
                r0 = pl.multiple_of(i * 8, 8)
                for part in range(2):
                    stripe(wot_hbm, wot_v, r0, part, 2, S_WO, 1)
                    stripe(wg_hbm, wg_v, r0 + 512, part, 2, S_WG, 1)
                return carry

            def mod_events(i, carry):
                r0 = pl.multiple_of(i * 8, 8)
                stripe(wmod_hbm, wmod_v, r0, 0, 1, S_MOD, 0)
                stripe(wmod_hbm, wmod_v, r0 + HALF, 0, 1, S_MOD, 1)
                return carry

            def wq_events(i, carry):
                r0 = pl.multiple_of(i * 8, 8)
                for part in range(2):
                    stripe(wq_hbm, wq_v, r0, part, 2, S_WQ, 0)
                    stripe(wq_hbm, wq_v, r0 + HALF, part, 2, S_WQ, 1)
                return carry

            small = [mk(c_hbm, c_v, sem.at[S_MOD]), mk(x_hbm, x_v, sem.at[S_MOD]), mk(wr_hbm, wr_v, sem.at[S_MOD])]
            with S("head"):
                lax.fori_loop(0, 8, prefix, 0)
                lax.fori_loop(0, HALF // 8, mod_events, 0)
                for cp in small:
                    cp.start()
                lax.fori_loop(0, HALF // 8, wq_events, 0)
            s_scr[...] = jnp.zeros_like(s_scr)

            def silu_c():
                cf = c_v[...].astype(F32)
                return (cf * _sigmoid(cf)).astype(BF16)

            def do_mod():
                for cp in small:
                    cp.wait()
                wait_all(wmod_v, S_MOD)
                mod_a = jnp.dot(silu_c(), wmod_v[:, 0:2 * D], preferred_element_type=F32)
                sa, ca = mod_a[:, 0:D], mod_a[:, D:2 * D]
                h_scr[...] = _layernorm(x_v[...].astype(F32)) * (1.0 + ca) + sa

            def do_mod_b(i):
                mb = jnp.dot(silu_c(), wmod_v[:, (2 + 2 * i) * D:(4 + 2 * i) * D], preferred_element_type=F32)
                mod_scr[2 * i] = mb[:, 0:D]
                mod_scr[2 * i + 1] = mb[:, D:2 * D]

            NQ = 2

            def do_q(i):
                if i == 0:
                    wait_all(wq_v, S_WQ)
                nh = Hkv // NQ
                q = jnp.dot(h_scr[...].astype(BF16), wq_v[:, i * nh * rep * Dh:(i + 1) * nh * rep * Dh],
                            preferred_element_type=F32)
                for t in range(nh):
                    q2 = jnp.concatenate([q[:, (rep * t + r) * Dh:(rep * t + r + 1) * Dh] for r in range(rep)], axis=0)
                    q_scr[i * nh + t] = q2.astype(BF16)

            def first_step(b, carry):
                for j in range(nev):
                    kv_event(0, b, j)
                work = {1: do_mod, 2: lambda: do_mod_b(0), 3: lambda: do_mod_b(1),
                        4: lambda: do_q(0), 5: lambda: do_q(1)}
                for bb, f in work.items():
                    pl.when(b == bb)(f)
                return carry

            with S("first"):
                lax.fori_loop(0, B, first_step, 0)

            row_s = lax.broadcasted_iota(jnp.int32, (M, ks), 0) % B
            row_o = lax.broadcasted_iota(jnp.int32, (M, Dh), 0) % B

            def qk_slice(h, b, g):
                cols = pl.ds(g * ks, ks)
                sn = lax.dot_general(q_scr[h], kbuf[h % 2, b, cols], _NT, preferred_element_type=F32)
                s_scr[:, cols] = jnp.where(row_s == b, sn, s_scr[:, cols])

            def pv_slice(h, b, g):
                cols = pl.ds(g * ks, ks)
                return jnp.dot(p_scr[:, cols], vbuf[h % NV, b, cols], preferred_element_type=F32)

            def softmax():
                s = s_scr[...] * scale
                m = jnp.max(s, axis=-1, keepdims=True)
                p = jnp.exp(s - m)
                l_scr[...] = jnp.broadcast_to(jnp.sum(p, axis=-1, keepdims=True), (M, Dh))
                p_scr[...] = p.astype(BF16)

            def phase(h, event, n_events, do_pv, unroll=False):
                if do_pv:
                    wait_all(vbuf.at[(h - 1) % NV], S_V + (h - 1) % NV)

                def step(b, o_acc):
                    @pl.when(b % (B // 2) == 0)
                    def _():
                        wait_all(kbuf.at[h % 2, pl.ds(b, B // 2)], S_K + (h % 2) * 2 + b // (B // 2))
                    o = None
                    e = 0
                    for g in range(2 * nsl):
                        e_end = (g + 1) * n_events // (2 * nsl)
                        for j in range(e, e_end):
                            event(b, j)
                        e = e_end
                        if g % 2 == 0:
                            qk_slice(h, b, g // 2)
                        elif do_pv:
                            d = pv_slice(h - 1, b, g // 2)
                            o = d if o is None else o + d
                    return jnp.where(row_o == b, o, o_acc) if do_pv else o_acc

                o_acc = lax.fori_loop(0, B, step, jnp.zeros((M, Dh), F32), unroll=unroll)
                if do_pv:
                    a_scr[h - 1] = o_acc / l_scr[...]
                softmax()

            with S("ph0"):
                phase(0, lambda b, j: kv_event(1, b, j), nev, False, unroll0)

            def main(h, carry):
                with S("ph"):
                    phase(h, lambda b, j: kv_event(h + 1, b, j), nev, True)
                return carry

            lax.fori_loop(1, Hkv - 1, main, 0)

            def wo_wu_event(b, j):
                r0 = pl.multiple_of(b * 64 + (j // 2) * 8, 8)
                stripe(wu_hbm, wu_v, r0, j % 2, 2, S_WU, 0)
                stripe(wot_hbm, wot_v, r0 + 64, j % 2, 2, S_WO, 1)

            with S("phlast"):
                phase(Hkv - 1, wo_wu_event, 16, True, unrolll)

            dpieces = [(0, 128), (128, 128), (256, 128), (384, 64), (448, 64)]

            def dsem(r):
                return S_FREE + [i for i, (s0, n) in enumerate(dpieces) if s0 <= r < s0 + n][0]

            def rows(src, dst, lo, hi, semf, prio):
                return [lambda r0=r0, part=part: stripe(src, dst, r0, part, 2, semf(r0), prio)
                        for r0 in range(lo, hi, 8) for part in range(2)]

            q0 = rows(wu_hbm, wu_v, 512, D, lambda r: S_WU, 0) + rows(wg_hbm, wg_v, 0, 288, lambda r: S_WG, 0)
            q1 = rows(wg_hbm, wg_v, 288, 512, lambda r: S_WG, 1)
            for s0, n in dpieces[:4]:
                q0 += rows(wdt_hbm, wdt_v, s0, s0 + n // 2, dsem, 0)
                q1 += rows(wdt_hbm, wdt_v, s0 + n // 2, s0 + n, dsem, 1)
            q1 += rows(wdt_hbm, wdt_v, 448, 512, dsem, 1)
            col = 0
            for gi, n in enumerate(cgroups):
                for _ in range(n):
                    idx = (pl.ds(512, D - 512), pl.ds(col, lastw))
                    q1.append(lambda idx=idx, gi=gi: mk(wdt_hbm.at[idx], wdt_v.at[idx], sem_last.at[gi]).start(priority=1))
                    col += lastw
            nevents = max(len(q0), len(q1))
            pos = [0]

            def advance_to(e):
                e = min(e, nevents)
                while pos[0] < e:
                    for q in (q0, q1):
                        if pos[0] < len(q):
                            q[pos[0]]()
                    pos[0] += 1

            def advance(n):
                advance_to(pos[0] + n)

            h = Hkv - 1
            wait_all(vbuf.at[h % NV], S_V + h % NV)
            o_acc = jnp.zeros((M, Dh), F32)
            with S("pvlast"):
                for b in range(B):
                    o = None
                    for g in range(nsl):
                        advance(4 // nsl)
                        d = pv_slice(h, b, g)
                        o = d if o is None else o + d
                    o_acc = jnp.where(row_o == b, o, o_acc)
                a_scr[h] = o_acc / l_scr[...]

            advance_to(sch["wo"])
            with S("w_wo"):
                wait_all(wot_v, S_WO)
            ao = None
            NO = 8
            for i in range(NO):
                nh = Hkv // NO
                parts = []
                for t in range(i * nh, (i + 1) * nh):
                    a = a_scr[t]
                    parts += [a[r * B:(r + 1) * B] for r in range(rep)]
                attn = jnp.concatenate(parts, axis=1).astype(BF16)
                n = nh * rep * Dh
                d = lax.dot_general(attn, wot_v[:, i * n:(i + 1) * n], _NT, preferred_element_type=F32)
                ao = d if ao is None else ao + d
                advance(sch["wo_step"])
            x1 = x_v[...].astype(F32) + mod_scr[0] * ao
            h2f = _layernorm(x1) * (1.0 + mod_scr[2]) + mod_scr[1]
            h2 = h2f.astype(BF16)
            wr = wr_v[...].astype(F32).reshape(1, D)
            gate_r = _sigmoid(jnp.sum(h2.astype(F32) * wr, axis=-1, keepdims=True))
            gb = mod_scr[3]
            advance(1)

            NF = 6
            nf = F // NF
            with S("w_u"):
                wait_all(wu_v, S_WU)
            us = []
            for i in range(NF):
                us.append(jnp.dot(h2, wu_v[:, i * nf:(i + 1) * nf], preferred_element_type=F32))
                advance(sch["u_step"])
            advance_to(sch["g"])
            with S("w_g"):
                wait_all(wg_v, S_WG)
            acts = []
            for i in range(NF):
                g = jnp.dot(h2, wg_v[:, i * nf:(i + 1) * nf], preferred_element_type=F32)
                acts.append((g * _sigmoid(g) * us[i]).astype(BF16))
                advance(sch["g_step"])
            act = jnp.concatenate(acts, axis=1)
            advance_to(nevents)

            def finish(s0, n, y):
                hh = h2f[:, s0:s0 + n]
                upd = hh * 0.0 + y * gate_r
                o_ref[:, s0:s0 + n] = (x1[:, s0:s0 + n] + gb[:, s0:s0 + n] * (hh + upd)).astype(o_ref.dtype)

            held = None
            for i, (s0, n) in enumerate(dpieces):
                with S("w_d%d" % s0):
                    wait_all(wdt_v.at[pl.ds(s0, n)], S_FREE + i)
                y = lax.dot_general(act, wdt_v[pl.ds(s0, n), :], _NT, preferred_element_type=F32)
                if n == 128:
                    finish(s0, n, y)
                elif held is None:
                    held = y
                else:
                    finish(s0 - 64, 128, jnp.concatenate([held, y], axis=1))
                    held = None
            return act, h2f[:, 512:], gate_r, x1[:, 512:], gb[:, 512:]

          if scoped:
            act, hh, gate_r, x1, gb = pl.run_scoped(body, pltpu.SemaphoreType.DMA((nsem,)))
          else:
            act, hh, gate_r, x1, gb = body(maybe_sem[0])
          y = None
          col = 0
          for gi, n in enumerate(cgroups):
            idx = (pl.ds(512, D - 512), pl.ds(col, n * lastw))
            with S("w_c%d" % col):
                mk(wdt_v.at[idx], wdt_v.at[idx], sem_last.at[gi]).wait()
            d = lax.dot_general(act[:, col:col + n * lastw], wdt_v[idx], _NT, preferred_element_type=F32)
            y = d if y is None else y + d
            col += n * lastw
          upd = hh * 0.0 + y * gate_r
          o_ref[:, 512:] = (x1 + gb * (hh + upd)).astype(o_ref.dtype)

        any_spec = pl.BlockSpec(memory_space=pl.ANY)
        out = pl.pallas_call(
            kernel,
            out_shape=jax.ShapeDtypeStruct((B, D), A_x.dtype),
            in_specs=[any_spec] * 11,
            out_specs=pl.BlockSpec(memory_space=pltpu.VMEM),
            scratch_shapes=[
                pltpu.VMEM((B, D), BF16), pltpu.VMEM((B, D), BF16), pltpu.VMEM((D,), BF16),
                pltpu.VMEM((D, 6 * D), BF16), pltpu.VMEM((D, Hq * Dh), BF16), pltpu.VMEM((D, Hq * Dh), BF16),
                pltpu.VMEM((D, F), BF16), pltpu.VMEM((D, F), BF16), pltpu.VMEM((D, F), BF16),
                pltpu.VMEM((2, B, W, Dh), BF16), pltpu.VMEM((NV, B, W, Dh), BF16),
                pltpu.VMEM((Hkv, M, Dh), BF16), pltpu.VMEM((Hkv, M, Dh), F32),
                pltpu.VMEM((M, W), F32), pltpu.VMEM((M, W), BF16), pltpu.VMEM((M, Dh), F32),
                pltpu.VMEM((B, D), F32), pltpu.VMEM((4, B, D), F32),
                pltpu.SemaphoreType.DMA((len(cgroups),)),
            ] + ([] if scoped else [pltpu.SemaphoreType.DMA((nsem,))]),
            compiler_params=pltpu.CompilerParams(vmem_limit_bytes=100 * 1024 * 1024,
                                                 disable_semaphore_checks=nosem, disable_bounds_checks=nobounds),
            name="adaln_attn_moe_decode",
        )(A_x.reshape(B, D), A_k_cache, A_v_cache, A_wq, A_wo.T, B_w_r, B_w_gate, B_w_up, B_w_down.T, c, w_mod)
        return out.reshape(B, Sq, D)
    return fn


_impl = make(ch=[208] + [248] * 7 + [104], vch=[168] + [256] * 7 + [88])


@jax.jit
def pallas_adaLN_cond__sliding_block_cached__moe_arch_mod__decode_kernel(
    A_x: jax.Array,
    A_k_cache: jax.Array,
    A_v_cache: jax.Array,
    A_wq: jax.Array,
    A_wo: jax.Array,
    B_x: jax.Array,
    B_w_r: jax.Array,
    B_w_gate: jax.Array,
    B_w_up: jax.Array,
    B_w_down: jax.Array,
    c: jax.Array,
    w_mod: jax.Array,
):
    return _impl(A_x, A_k_cache, A_v_cache, A_wq, A_wo, B_x, B_w_r, B_w_gate, B_w_up, B_w_down, c, w_mod)
```

```python
import contextlib
import jax
import jax.numpy as jnp
from jax import lax
import jax.experimental.pallas as pl
import jax.experimental.pallas.tpu as pltpu

F32 = jnp.float32
BF16 = jnp.bfloat16
_NT = (((1,), (1,)), ((), ()))
TR, TC = 8, 128


def _layernorm(x, eps=1e-05):
    m = jnp.mean(x, axis=-1, keepdims=True)
    d = x - m
    v = jnp.mean(d * d, axis=-1, keepdims=True)
    return d / jnp.sqrt(v + eps)


def _sigmoid(x):
    return 1.0 / (1.0 + jnp.exp(-x))


def _cuts(lo, hi, phase, pattern):
    period = sum(pattern)
    pts, t = [], phase - period * (phase // period + 1)
    while t < hi:
        for n in pattern:
            if lo < t < hi:
                pts.append(t)
            t += n
    pts = [lo] + pts + [hi]
    return list(zip(pts[:-1], pts[1:]))


def _rects(t0, t1, ncol, split):
    out = []
    while t0 < t1:
        s, c = divmod(t0, ncol)
        n = min(ncol - c, t1 - t0)
        out.append((s * TR, c * TC, n * TC))
        t0 += n
    if split and len(out) == 1 and out[0][2] >= 2 * TC:
        r, c, n = out[0]
        half = n // (2 * TC) * TC
        out = [(r, c, half), (r, c + half, n - half)]
    return out


def make(ev, ks=1024, scopes=False, sched=None, ph=None, p0=(31,) * 8 + (8,), p1=(32,), d0=4, d1=-1,
         split=True, gsplit=1177, dsplit=216):
    S = (lambda n: jax.named_scope(n)) if scopes else (lambda n: contextlib.nullcontext())
    sch = dict(wo=102, wo_step=1.5, u=115, u_step=1, g=146, g_step=1, pv_step=1)
    sch.update(sched or {})
    phase_of = dict(mod=22, wq=22, wo=22, wg=30, wu=30, wd=30)
    phase_of.update(ph or {})

    def fn(A_x, A_k_cache, A_v_cache, A_wq, A_wo, B_x, B_w_r, B_w_gate, B_w_up, B_w_down, c, w_mod):
        B, Sq, D = A_x.shape
        _, Hkv, Sk, Dh = A_k_cache.shape
        Hq = A_wq.shape[1] // Dh
        rep = Hq // Hkv
        F = B_w_gate.shape[1]
        W = min(4096, max(256, Sk // 4))
        assert Sq == 1 and rep == 2 and B == 8 and D == 576
        scale = Dh ** (-0.5)
        M = rep * B
        for which in range(2):
            cover = sorted((o, n) for e in ev for (w, o, n, p) in e if w == which)
            assert cover[0][0] == 0 and all(a[0] + a[1] == b[0] for a, b in zip(cover, cover[1:])) and sum(n for _, n in cover) == W
        nev = len(ev)
        nsl = W // ks
        NV = 4
        S_WO, S_WG, S_WU, S_MOD, S_WQ, S_K, S_V = 0, 1, 2, 3, 4, 5, 9
        S_WD = S_V + NV
        dpieces = [(0, 128), (256, 128), (128, 64), (384, 64), (192, 64), (448, 64), (512, 64)]
        nsem = S_WD + len(dpieces)

        def kernel(x_hbm, k_hbm, v_hbm, wq_hbm, wot_hbm, wr_hbm, wg_hbm, wu_hbm, wdt_hbm, c_hbm, wmod_hbm,
                   o_ref,
                   x_v, c_v, wr_v, wmod_v, wq_v, wot_v, wg_v, wu_v, wdt_v, kbuf, vbuf,
                   q_scr, a_scr, s_scr, p_scr, l_scr, h_scr, mod_scr):
          mk = pltpu.make_async_copy

          def body(sem):
            def wait_all(dst, i):
                mk(dst, dst, sem.at[i]).wait()

            def chunks(src, dst, name, semf, queue, lo=0, hi=None):
                ncol = src.shape[1] // TC
                hi = src.shape[0] // TR * ncol if hi is None else hi
                cuts = (_cuts(lo, hi, phase_of[name] + d0, p0) if queue == 0
                        else _cuts(lo, hi, phase_of[name] + d1, p1))

                def start(t0, t1):
                    for r, c0, n in _rects(t0, t1, ncol, split and queue == 1):
                        idx = (pl.ds(r, TR), pl.ds(c0, n))
                        mk(src.at[idx], dst.at[idx], sem.at[semf(r)]).start(priority=queue)
                return [(lambda t0=t0, t1=t1: start(t0, t1), {semf(r) for r, _, _ in _rects(t0, t1, ncol, False)})
                        for t0, t1 in cuts]

            class Stream:
                def __init__(self, q0, q1):
                    self.q0, self.q1, self.pos = q0, q1, 0
                    self.n = max(len(q0), len(q1))

                def advance_to(self, e):
                    while self.pos < min(e, self.n):
                        for q in (self.q0, self.q1):
                            if self.pos < len(q):
                                q[self.pos][0]()
                        self.pos += 1

                def wait(self, dst, i):
                    last = max(n for q in (self.q0, self.q1) for n, (_, sems) in enumerate(q) if i in sems)
                    self.advance_to(last + 1)
                    wait_all(dst, i)

            def kv_event(h, b, j):
                for which, rows, n, prio in ev[j]:
                    if which == 0:
                        mk(k_hbm.at[b, h, pl.ds(Sk - W + rows, n), :], kbuf.at[h % 2, b, pl.ds(rows, n)],
                           sem.at[S_K + (h % 2) * 2 + b // (B // 2)]).start(priority=prio)
                    else:
                        mk(v_hbm.at[b, h, pl.ds(Sk - W + rows, n), :], vbuf.at[h % NV, b, pl.ds(rows, n)],
                           sem.at[S_V + h % NV]).start(priority=prio)

            small = [mk(c_hbm, c_v, sem.at[S_MOD]), mk(x_hbm, x_v, sem.at[S_MOD]), mk(wr_hbm, wr_v, sem.at[S_MOD])]
            with S("head"):
                q0 = chunks(wmod_hbm, wmod_v, "mod", lambda r: S_MOD, 0)
                q1 = chunks(wq_hbm, wq_v, "wq", lambda r: S_WQ, 1)
                lead = len(q1) - len(q0)
                for f, _ in q1[:lead]:
                    f()
                head = Stream(q0, q1[lead:])
                head.advance_to(20)
                for cp in small:
                    cp.start()
                head.advance_to(head.n)
            s_scr[...] = jnp.zeros_like(s_scr)

            def silu_c():
                cf = c_v[...].astype(F32)
                return (cf * _sigmoid(cf)).astype(BF16)

            def do_mod():
                for cp in small:
                    cp.wait()
                wait_all(wmod_v, S_MOD)
                mod_a = jnp.dot(silu_c(), wmod_v[:, 0:2 * D], preferred_element_type=F32)
                sa, ca = mod_a[:, 0:D], mod_a[:, D:2 * D]
                h_scr[...] = _layernorm(x_v[...].astype(F32)) * (1.0 + ca) + sa

            def do_mod_b(i):
                mb = jnp.dot(silu_c(), wmod_v[:, (2 + 2 * i) * D:(4 + 2 * i) * D], preferred_element_type=F32)
                mod_scr[2 * i] = mb[:, 0:D]
                mod_scr[2 * i + 1] = mb[:, D:2 * D]

            NQ = 2

            def do_q(i):
                if i == 0:
                    wait_all(wq_v, S_WQ)
                nh = Hkv // NQ
                q = jnp.dot(h_scr[...].astype(BF16), wq_v[:, i * nh * rep * Dh:(i + 1) * nh * rep * Dh],
                            preferred_element_type=F32)
                for t in range(nh):
                    q2 = jnp.concatenate([q[:, (rep * t + r) * Dh:(rep * t + r + 1) * Dh] for r in range(rep)], axis=0)
                    q_scr[i * nh + t] = q2.astype(BF16)

            def first_step(b, carry):
                for j in range(nev):
                    kv_event(0, b, j)
                work = {2: do_mod, 3: lambda: do_mod_b(0), 4: lambda: do_mod_b(1),
                        5: lambda: do_q(0), 6: lambda: do_q(1)}
                for bb, f in work.items():
                    pl.when(b == bb)(f)
                return carry

            with S("first"):
                lax.fori_loop(0, B, first_step, 0)

            row_s = lax.broadcasted_iota(jnp.int32, (M, ks), 0) % B
            row_o = lax.broadcasted_iota(jnp.int32, (M, Dh), 0) % B

            def qk_slice(h, b, g):
                cols = pl.ds(g * ks, ks)
                sn = lax.dot_general(q_scr[h], kbuf[h % 2, b, cols], _NT, preferred_element_type=F32)
                s_scr[:, cols] = jnp.where(row_s == b, sn, s_scr[:, cols])

            def pv_slice(h, b, g):
                cols = pl.ds(g * ks, ks)
                return jnp.dot(p_scr[:, cols], vbuf[h % NV, b, cols], preferred_element_type=F32)

            def softmax():
                s = s_scr[...] * scale
                m = jnp.max(s, axis=-1, keepdims=True)
                p = jnp.exp(s - m)
                l_scr[...] = jnp.broadcast_to(jnp.sum(p, axis=-1, keepdims=True), (M, Dh))
                p_scr[...] = p.astype(BF16)

            def phase(h, event, do_pv, static=False):
                if do_pv:
                    wait_all(vbuf.at[(h - 1) % NV], S_V + (h - 1) % NV)

                def step(b, o_acc):
                    def wait_k():
                        wait_all(kbuf.at[h % 2, pl.ds(b, B // 2)], S_K + (h % 2) * 2 + b // (B // 2))
                    if not static:
                        pl.when(b % (B // 2) == 0)(wait_k)
                    elif b % (B // 2) == 0:
                        wait_k()
                    o = None
                    e = 0
                    for g in range(2 * nsl):
                        e_end = (g + 1) * nev // (2 * nsl)
                        for j in range(e, e_end):
                            event(b, j)
                        e = e_end
                        if g % 2 == 0:
                            qk_slice(h, b, g // 2)
                        elif do_pv:
                            d = pv_slice(h - 1, b, g // 2)
                            o = d if o is None else o + d
                    return jnp.where(row_o == b, o, o_acc) if do_pv else o_acc

                o_acc = jnp.zeros((M, Dh), F32)
                if static:
                    for b in range(B):
                        o_acc = step(b, o_acc)
                else:
                    o_acc = lax.fori_loop(0, B, step, o_acc)
                if do_pv:
                    a_scr[h - 1] = o_acc / l_scr[...]
                softmax()

            with S("ph0"):
                phase(0, lambda b, j: kv_event(1, b, j), False)

            def main(h, carry):
                with S("ph"):
                    phase(h, lambda b, j: kv_event(h + 1, b, j), True)
                return carry

            lax.fori_loop(1, Hkv - 1, main, 0)

            def dsem(r):
                return S_WD + [i for i, (s0, n) in enumerate(dpieces) if s0 <= r < s0 + n][0]

            dcut = dsplit // TR * (F // TC)
            tail = Stream(
                chunks(wu_hbm, wu_v, "wu", lambda r: S_WU, 0)
                + chunks(wg_hbm, wg_v, "wg", lambda r: S_WG, 0, hi=gsplit)
                + chunks(wdt_hbm, wdt_v, "wd", dsem, 0, hi=dcut),
                chunks(wot_hbm, wot_v, "wo", lambda r: S_WO, 1)
                + chunks(wg_hbm, wg_v, "wg", lambda r: S_WG, 1, lo=gsplit)
                + chunks(wdt_hbm, wdt_v, "wd", dsem, 1, lo=dcut))

            with S("phlast"):
                phase(Hkv - 1, lambda b, j: tail.advance_to(tail.pos + 1), True, static=True)

            h = Hkv - 1
            wait_all(vbuf.at[h % NV], S_V + h % NV)
            o_acc = jnp.zeros((M, Dh), F32)
            with S("pvlast"):
                for b in range(B):
                    o = None
                    for g in range(nsl):
                        tail.advance_to(tail.pos + sch["pv_step"])
                        d = pv_slice(h, b, g)
                        o = d if o is None else o + d
                    o_acc = jnp.where(row_o == b, o, o_acc)
                a_scr[h] = o_acc / l_scr[...]

            tail.advance_to(sch["wo"])
            with S("w_wo"):
                tail.wait(wot_v, S_WO)
            ao = None
            NO = 8
            for i in range(NO):
                nh = Hkv // NO
                parts = []
                for t in range(i * nh, (i + 1) * nh):
                    a = a_scr[t]
                    parts += [a[r * B:(r + 1) * B] for r in range(rep)]
                attn = jnp.concatenate(parts, axis=1).astype(BF16)
                n = nh * rep * Dh
                d = lax.dot_general(attn, wot_v[:, i * n:(i + 1) * n], _NT, preferred_element_type=F32)
                ao = d if ao is None else ao + d
                tail.advance_to(sch["wo"] + (i + 1) * sch["wo_step"])
            x1 = x_v[...].astype(F32) + mod_scr[0] * ao
            h2f = _layernorm(x1) * (1.0 + mod_scr[2]) + mod_scr[1]
            h2 = h2f.astype(BF16)
            wr = wr_v[...].astype(F32).reshape(1, D)
            gate_r = _sigmoid(jnp.sum(h2.astype(F32) * wr, axis=-1, keepdims=True))
            gb = mod_scr[3]

            NF = 6
            nf = F // NF
            tail.advance_to(sch["u"])
            with S("w_u"):
                tail.wait(wu_v, S_WU)
            us = []
            for i in range(NF):
                us.append(jnp.dot(h2, wu_v[:, i * nf:(i + 1) * nf], preferred_element_type=F32))
                tail.advance_to(sch["u"] + (i + 1) * sch["u_step"])
            tail.advance_to(sch["g"])
            with S("w_g"):
                tail.wait(wg_v, S_WG)
            acts = []
            for i in range(NF):
                g = jnp.dot(h2, wg_v[:, i * nf:(i + 1) * nf], preferred_element_type=F32)
                acts.append((g * _sigmoid(g) * us[i]).astype(BF16))
                tail.advance_to(sch["g"] + (i + 1) * sch["g_step"])
            act = jnp.concatenate(acts, axis=1)
            tail.advance_to(tail.n)

            def finish(s0, n, y):
                hh = h2f[:, s0:s0 + n]
                upd = hh * 0.0 + y * gate_r
                o_ref[:, s0:s0 + n] = (x1[:, s0:s0 + n] + gb[:, s0:s0 + n] * (hh + upd)).astype(o_ref.dtype)

            held = {}
            for i, (s0, n) in enumerate(dpieces):
                with S("w_d%d" % s0):
                    tail.wait(wdt_v.at[pl.ds(s0, n)], S_WD + i)
                y = lax.dot_general(act, wdt_v[pl.ds(s0, n), :], _NT, preferred_element_type=F32)
                if s0 % TC:
                    finish(s0 - n, 2 * n, jnp.concatenate([held.pop(s0 - n), y], axis=1))
                elif n == TC or s0 + n == D:
                    finish(s0, n, y)
                else:
                    held[s0] = y
            assert not held

          pl.run_scoped(body, pltpu.SemaphoreType.DMA((nsem,)))

        any_spec = pl.BlockSpec(memory_space=pl.ANY)
        out = pl.pallas_call(
            kernel,
            out_shape=jax.ShapeDtypeStruct((B, D), A_x.dtype),
            in_specs=[any_spec] * 11,
            out_specs=pl.BlockSpec(memory_space=pltpu.VMEM),
            scratch_shapes=[
                pltpu.VMEM((B, D), BF16), pltpu.VMEM((B, D), BF16), pltpu.VMEM((D,), BF16),
                pltpu.VMEM((D, 6 * D), BF16), pltpu.VMEM((D, Hq * Dh), BF16), pltpu.VMEM((D, Hq * Dh), BF16),
                pltpu.VMEM((D, F), BF16), pltpu.VMEM((D, F), BF16), pltpu.VMEM((D, F), BF16),
                pltpu.VMEM((2, B, W, Dh), BF16), pltpu.VMEM((NV, B, W, Dh), BF16),
                pltpu.VMEM((Hkv, M, Dh), BF16), pltpu.VMEM((Hkv, M, Dh), F32),
                pltpu.VMEM((M, W), F32), pltpu.VMEM((M, W), BF16), pltpu.VMEM((M, Dh), F32),
                pltpu.VMEM((B, D), F32), pltpu.VMEM((4, B, D), F32),
            ],
            compiler_params=pltpu.CompilerParams(vmem_limit_bytes=100 * 1024 * 1024),
            name="adaln_attn_moe_decode",
        )(A_x.reshape(B, D), A_k_cache, A_v_cache, A_wq, A_wo.T, B_w_r, B_w_gate, B_w_up, B_w_down.T, c, w_mod)
        return out.reshape(B, Sq, D)
    return fn


_impl = make(ev=[[(0, 0, 208, 0), (1, 1960, 88, 1)], [(0, 208, 248, 0), (1, 0, 168, 1)], [(0, 456, 248, 0), (1, 168, 256, 1)], [(0, 704, 248, 0), (1, 424, 256, 1)], [(0, 952, 248, 0), (1, 680, 256, 1)], [(0, 1200, 248, 0), (1, 936, 256, 1)], [(0, 1448, 248, 0), (1, 1192, 256, 1)], [(0, 1696, 248, 0), (1, 1448, 256, 1)], [(0, 1944, 104, 0), (1, 1704, 256, 1)]], d1=-2)


@jax.jit
def pallas_adaLN_cond__sliding_block_cached__moe_arch_mod__decode_kernel(
    A_x: jax.Array,
    A_k_cache: jax.Array,
    A_v_cache: jax.Array,
    A_wq: jax.Array,
    A_wo: jax.Array,
    B_x: jax.Array,
    B_w_r: jax.Array,
    B_w_gate: jax.Array,
    B_w_up: jax.Array,
    B_w_down: jax.Array,
    c: jax.Array,
    w_mod: jax.Array,
):
    return _impl(A_x, A_k_cache, A_v_cache, A_wq, A_wo, B_x, B_w_r, B_w_gate, B_w_up, B_w_down, c, w_mod)
```

```python
import contextlib
import jax
import jax.numpy as jnp
from jax import lax
import jax.experimental.pallas as pl
import jax.experimental.pallas.tpu as pltpu

F32 = jnp.float32
BF16 = jnp.bfloat16
_NT = (((1,), (1,)), ((), ()))
TR, TC = 8, 128


def _layernorm(x, eps=1e-05):
    m = jnp.mean(x, axis=-1, keepdims=True)
    d = x - m
    v = jnp.mean(d * d, axis=-1, keepdims=True)
    return d / jnp.sqrt(v + eps)


def _sigmoid(x):
    return 1.0 / (1.0 + jnp.exp(-x))


def _cuts(lo, hi, phase, pattern):
    period = sum(pattern)
    pts, t = [], phase - period * (phase // period + 1)
    while t < hi:
        for n in pattern:
            if lo < t < hi:
                pts.append(t)
            t += n
    pts = [lo] + pts + [hi]
    return list(zip(pts[:-1], pts[1:]))


def _rects(t0, t1, ncol, split):
    out = []
    while t0 < t1:
        s, c = divmod(t0, ncol)
        n = min(ncol - c, t1 - t0)
        out.append((s * TR, c * TC, n * TC))
        t0 += n
    if split and len(out) == 1 and out[0][2] >= 2 * TC:
        r, c, n = out[0]
        half = n // (2 * TC) * TC
        out = [(r, c, half), (r, c + half, n - half)]
    return out


def make(ev, ks=1024, scopes=False, sched=None, ph=None, p0=(31,) * 8 + (8,), p1=(32,), d0=4, d1=-1,
         split=True, gsplit=1177, dsplit=216, last=0, wrem=False, t0=24, t1=22, worder='rkv', lead_extra=0):
    S = (lambda n: jax.named_scope(n)) if scopes else (lambda n: contextlib.nullcontext())
    sch = dict(wo=102, wo_step=1.5, u=115, u_step=1, g=146, g_step=1, pv_step=1)
    sch.update(sched or {})
    phase_of = dict(mod=22, wq=22, wo=22, wg=30, wu=30, wd=30)
    phase_of.update(ph or {})

    def fn(A_x, A_k_cache, A_v_cache, A_wq, A_wo, B_x, B_w_r, B_w_gate, B_w_up, B_w_down, c, w_mod):
        B, Sq, D = A_x.shape
        _, Hkv, Sk, Dh = A_k_cache.shape
        Hq = A_wq.shape[1] // Dh
        rep = Hq // Hkv
        F = B_w_gate.shape[1]
        W = min(4096, max(256, Sk // 4))
        assert Sq == 1 and rep == 2 and B == 8 and D == 576
        scale = Dh ** (-0.5)
        M = rep * B
        for which in range(2):
            cover = sorted((o, n) for e in ev for (w, o, n, p) in e if w == which)
            assert cover[0][0] == 0 and all(a[0] + a[1] == b[0] for a, b in zip(cover, cover[1:])) and sum(n for _, n in cover) == W
        nev = len(ev)
        nsl = W // ks
        NV = 4
        S_WO, S_WG, S_WU, S_MOD, S_WQ, S_K, S_V = 0, 1, 2, 3, 4, 5, 9
        S_WD = S_V + NV
        dpieces = [(0, 128), (256, 128), (128, 64), (384, 64), (192, 64), (448, 64)]
        dpieces += [(512 + last, 64 - last), (512, last)] if last else [(512, 64)]
        nsem = S_WD + len(dpieces)

        def kernel(x_hbm, k_hbm, v_hbm, wq_hbm, wot_hbm, wr_hbm, wg_hbm, wu_hbm, wdt_hbm, c_hbm, wmod_hbm,
                   o_ref,
                   x_v, c_v, wr_v, wmod_v, wq_v, wot_v, wg_v, wu_v, wdt_v, kbuf, vbuf,
                   q_scr, a_scr, s_scr, p_scr, l_scr, h_scr, mod_scr):
          mk = pltpu.make_async_copy

          def body(sem):
            def wait_all(dst, i):
                mk(dst, dst, sem.at[i]).wait()

            def chunks(src, dst, name, semf, queue, lo=0, hi=None):
                ncol = src.shape[1] // TC
                hi = src.shape[0] // TR * ncol if hi is None else hi
                if wrem:
                    cuts = _cuts(lo, hi, phase_of[name] - 22 + (t0, t1)[queue], (32,))
                else:
                    cuts = (_cuts(lo, hi, phase_of[name] + d0, p0) if queue == 0
                            else _cuts(lo, hi, phase_of[name] + d1, p1))

                def start(t0, t1, q, two):
                    for r, c0, n in _rects(t0, t1, ncol, two):
                        idx = (pl.ds(r, TR), pl.ds(c0, n))
                        mk(src.at[idx], dst.at[idx], sem.at[semf(r)]).start(priority=q)
                out = []
                for a, b in cuts:
                    sems = {semf(r) for r, _, _ in _rects(a, b, ncol, False)}
                    if wrem and queue == 0:
                        m = min(a + 1, b)
                        out.append(((lambda a=a, m=m: start(a, m, 1, False)), (lambda m=m, b=b: start(m, b, 0, False)), sems))
                    else:
                        out.append((None, (lambda a=a, b=b: start(a, b, queue, split and queue == 1)), sems))
                return out

            class Stream:
                def __init__(self, q0, q1):
                    self.q0, self.q1, self.pos = q0, q1, 0
                    self.n = max(len(q0), len(q1))

                def advance_to(self, e):
                    while self.pos < min(e, self.n):
                        d = {}
                        if self.pos < len(self.q0):
                            d["r"], d["k"], _ = self.q0[self.pos]
                        if self.pos < len(self.q1):
                            d["v"] = self.q1[self.pos][1]
                        for ch in worder:
                            if d.get(ch) is not None:
                                d[ch]()
                        self.pos += 1

                def wait(self, dst, i):
                    last = max(n for q in (self.q0, self.q1) for n, x in enumerate(q) if i in x[2])
                    self.advance_to(last + 1)
                    wait_all(dst, i)

            def kv_event(h, b, j):
                for which, rows, n, prio in ev[j]:
                    if which == 0:
                        mk(k_hbm.at[b, h, pl.ds(Sk - W + rows, n), :], kbuf.at[h % 2, b, pl.ds(rows, n)],
                           sem.at[S_K + (h % 2) * 2 + b // (B // 2)]).start(priority=prio)
                    else:
                        mk(v_hbm.at[b, h, pl.ds(Sk - W + rows, n), :], vbuf.at[h % NV, b, pl.ds(rows, n)],
                           sem.at[S_V + h % NV]).start(priority=prio)

            small = [mk(c_hbm, c_v, sem.at[S_MOD]), mk(x_hbm, x_v, sem.at[S_MOD]), mk(wr_hbm, wr_v, sem.at[S_MOD])]
            with S("head"):
                cut = wmod_hbm.shape[0] // TR * (wmod_hbm.shape[1] // TC) - 32 * lead_extra
                q0 = chunks(wmod_hbm, wmod_v, "mod", lambda r: S_MOD, 0, hi=cut)
                q1 = (chunks(wmod_hbm, wmod_v, "mod", lambda r: S_MOD, 1, lo=cut) if lead_extra else [])
                q1 += chunks(wq_hbm, wq_v, "wq", lambda r: S_WQ, 1)
                lead = len(q1) - len(q0)
                for x in q1[:lead]:
                    x[1]()
                head = Stream(q0, q1[lead:])
                head.advance_to(20)
                for cp in small:
                    cp.start()
                head.advance_to(head.n)
            s_scr[...] = jnp.zeros_like(s_scr)

            def silu_c():
                cf = c_v[...].astype(F32)
                return (cf * _sigmoid(cf)).astype(BF16)

            def do_mod():
                for cp in small:
                    cp.wait()
                wait_all(wmod_v, S_MOD)
                mod_a = jnp.dot(silu_c(), wmod_v[:, 0:2 * D], preferred_element_type=F32)
                sa, ca = mod_a[:, 0:D], mod_a[:, D:2 * D]
                h_scr[...] = _layernorm(x_v[...].astype(F32)) * (1.0 + ca) + sa

            def do_mod_b(i):
                mb = jnp.dot(silu_c(), wmod_v[:, (2 + 2 * i) * D:(4 + 2 * i) * D], preferred_element_type=F32)
                mod_scr[2 * i] = mb[:, 0:D]
                mod_scr[2 * i + 1] = mb[:, D:2 * D]

            NQ = 2

            def do_q(i):
                if i == 0:
                    wait_all(wq_v, S_WQ)
                nh = Hkv // NQ
                q = jnp.dot(h_scr[...].astype(BF16), wq_v[:, i * nh * rep * Dh:(i + 1) * nh * rep * Dh],
                            preferred_element_type=F32)
                for t in range(nh):
                    q2 = jnp.concatenate([q[:, (rep * t + r) * Dh:(rep * t + r + 1) * Dh] for r in range(rep)], axis=0)
                    q_scr[i * nh + t] = q2.astype(BF16)

            def first_step(b, carry):
                for j in range(nev):
                    kv_event(0, b, j)
                work = {2: do_mod, 3: lambda: do_mod_b(0), 4: lambda: do_mod_b(1),
                        5: lambda: do_q(0), 6: lambda: do_q(1)}
                for bb, f in work.items():
                    pl.when(b == bb)(f)
                return carry

            with S("first"):
                lax.fori_loop(0, B, first_step, 0)

            row_s = lax.broadcasted_iota(jnp.int32, (M, ks), 0) % B
            row_o = lax.broadcasted_iota(jnp.int32, (M, Dh), 0) % B

            def qk_slice(h, b, g):
                cols = pl.ds(g * ks, ks)
                sn = lax.dot_general(q_scr[h], kbuf[h % 2, b, cols], _NT, preferred_element_type=F32)
                s_scr[:, cols] = jnp.where(row_s == b, sn, s_scr[:, cols])

            def pv_slice(h, b, g):
                cols = pl.ds(g * ks, ks)
                return jnp.dot(p_scr[:, cols], vbuf[h % NV, b, cols], preferred_element_type=F32)

            def softmax():
                s = s_scr[...] * scale
                m = jnp.max(s, axis=-1, keepdims=True)
                p = jnp.exp(s - m)
                l_scr[...] = jnp.broadcast_to(jnp.sum(p, axis=-1, keepdims=True), (M, Dh))
                p_scr[...] = p.astype(BF16)

            def phase(h, event, do_pv, static=False):
                if do_pv:
                    wait_all(vbuf.at[(h - 1) % NV], S_V + (h - 1) % NV)

                def step(b, o_acc):
                    def wait_k():
                        wait_all(kbuf.at[h % 2, pl.ds(b, B // 2)], S_K + (h % 2) * 2 + b // (B // 2))
                    if not static:
                        pl.when(b % (B // 2) == 0)(wait_k)
                    elif b % (B // 2) == 0:
                        wait_k()
                    o = None
                    e = 0
                    for g in range(2 * nsl):
                        e_end = (g + 1) * nev // (2 * nsl)
                        for j in range(e, e_end):
                            event(b, j)
                        e = e_end
                        if g % 2 == 0:
                            qk_slice(h, b, g // 2)
                        elif do_pv:
                            d = pv_slice(h - 1, b, g // 2)
                            o = d if o is None else o + d
                    return jnp.where(row_o == b, o, o_acc) if do_pv else o_acc

                o_acc = jnp.zeros((M, Dh), F32)
                if static:
                    for b in range(B):
                        o_acc = step(b, o_acc)
                else:
                    o_acc = lax.fori_loop(0, B, step, o_acc)
                if do_pv:
                    a_scr[h - 1] = o_acc / l_scr[...]
                softmax()

            with S("ph0"):
                phase(0, lambda b, j: kv_event(1, b, j), False)

            def main(h, carry):
                with S("ph"):
                    phase(h, lambda b, j: kv_event(h + 1, b, j), True)
                return carry

            lax.fori_loop(1, Hkv - 1, main, 0)

            def dsem(r):
                return S_WD + [i for i, (s0, n) in enumerate(dpieces) if s0 <= r < s0 + n][0]

            dcut = dsplit // TR * (F // TC)
            tail = Stream(
                chunks(wu_hbm, wu_v, "wu", lambda r: S_WU, 0)
                + chunks(wg_hbm, wg_v, "wg", lambda r: S_WG, 0, hi=gsplit)
                + chunks(wdt_hbm, wdt_v, "wd", dsem, 0, hi=dcut),
                chunks(wot_hbm, wot_v, "wo", lambda r: S_WO, 1)
                + chunks(wg_hbm, wg_v, "wg", lambda r: S_WG, 1, lo=gsplit)
                + (chunks(wdt_hbm, wdt_v, "wd", dsem, 1, lo=dcut) if not last else
                   chunks(wdt_hbm, wdt_v, "wd", dsem, 1, lo=dcut, hi=64 * 36)
                   + chunks(wdt_hbm, wdt_v, "wd", dsem, 1, lo=(512 + last) // 8 * 36)
                   + chunks(wdt_hbm, wdt_v, "wd", dsem, 1, lo=64 * 36, hi=(512 + last) // 8 * 36)))

            with S("phlast"):
                phase(Hkv - 1, lambda b, j: tail.advance_to(tail.pos + 1), True, static=True)

            h = Hkv - 1
            wait_all(vbuf.at[h % NV], S_V + h % NV)
            o_acc = jnp.zeros((M, Dh), F32)
            with S("pvlast"):
                for b in range(B):
                    o = None
                    for g in range(nsl):
                        tail.advance_to(tail.pos + sch["pv_step"])
                        d = pv_slice(h, b, g)
                        o = d if o is None else o + d
                    o_acc = jnp.where(row_o == b, o, o_acc)
                a_scr[h] = o_acc / l_scr[...]

            tail.advance_to(sch["wo"])
            with S("w_wo"):
                tail.wait(wot_v, S_WO)
            ao = None
            NO = 8
            for i in range(NO):
                nh = Hkv // NO
                parts = []
                for t in range(i * nh, (i + 1) * nh):
                    a = a_scr[t]
                    parts += [a[r * B:(r + 1) * B] for r in range(rep)]
                attn = jnp.concatenate(parts, axis=1).astype(BF16)
                n = nh * rep * Dh
                d = lax.dot_general(attn, wot_v[:, i * n:(i + 1) * n], _NT, preferred_element_type=F32)
                ao = d if ao is None else ao + d
                tail.advance_to(sch["wo"] + (i + 1) * sch["wo_step"])
            x1 = x_v[...].astype(F32) + mod_scr[0] * ao
            h2f = _layernorm(x1) * (1.0 + mod_scr[2]) + mod_scr[1]
            h2 = h2f.astype(BF16)
            wr = wr_v[...].astype(F32).reshape(1, D)
            gate_r = _sigmoid(jnp.sum(h2.astype(F32) * wr, axis=-1, keepdims=True))
            gb = mod_scr[3]

            NF = 6
            nf = F // NF
            tail.advance_to(sch["u"])
            with S("w_u"):
                tail.wait(wu_v, S_WU)
            us = []
            for i in range(NF):
                us.append(jnp.dot(h2, wu_v[:, i * nf:(i + 1) * nf], preferred_element_type=F32))
                tail.advance_to(sch["u"] + (i + 1) * sch["u_step"])
            tail.advance_to(sch["g"])
            with S("w_g"):
                tail.wait(wg_v, S_WG)
            acts = []
            for i in range(NF):
                g = jnp.dot(h2, wg_v[:, i * nf:(i + 1) * nf], preferred_element_type=F32)
                acts.append((g * _sigmoid(g) * us[i]).astype(BF16))
                tail.advance_to(sch["g"] + (i + 1) * sch["g_step"])
            act = jnp.concatenate(acts, axis=1)
            tail.advance_to(tail.n)

            def finish(s0, n, y):
                hh = h2f[:, s0:s0 + n]
                upd = hh * 0.0 + y * gate_r
                o_ref[:, s0:s0 + n] = (x1[:, s0:s0 + n] + gb[:, s0:s0 + n] * (hh + upd)).astype(o_ref.dtype)

            held = {}
            for i, (s0, n) in enumerate(dpieces):
                with S("w_d%d" % s0):
                    tail.wait(wdt_v.at[pl.ds(s0, n)], S_WD + i)
                y = lax.dot_general(act, wdt_v[pl.ds(s0, n), :], _NT, preferred_element_type=F32)
                if last and s0 > 512:
                    held[s0] = y
                elif last and s0 == 512:
                    finish(512, 64, jnp.concatenate([y, held.pop(512 + last)], axis=1))
                elif s0 % TC:
                    finish(s0 - n, 2 * n, jnp.concatenate([held.pop(s0 - n), y], axis=1))
                elif n == TC or s0 + n == D:
                    finish(s0, n, y)
                else:
                    held[s0] = y
            assert not held

          pl.run_scoped(body, pltpu.SemaphoreType.DMA((nsem,)))

        any_spec = pl.BlockSpec(memory_space=pl.ANY)
        out = pl.pallas_call(
            kernel,
            out_shape=jax.ShapeDtypeStruct((B, D), A_x.dtype),
            in_specs=[any_spec] * 11,
            out_specs=pl.BlockSpec(memory_space=pltpu.VMEM),
            scratch_shapes=[
                pltpu.VMEM((B, D), BF16), pltpu.VMEM((B, D), BF16), pltpu.VMEM((D,), BF16),
                pltpu.VMEM((D, 6 * D), BF16), pltpu.VMEM((D, Hq * Dh), BF16), pltpu.VMEM((D, Hq * Dh), BF16),
                pltpu.VMEM((D, F), BF16), pltpu.VMEM((D, F), BF16), pltpu.VMEM((D, F), BF16),
                pltpu.VMEM((2, B, W, Dh), BF16), pltpu.VMEM((NV, B, W, Dh), BF16),
                pltpu.VMEM((Hkv, M, Dh), BF16), pltpu.VMEM((Hkv, M, Dh), F32),
                pltpu.VMEM((M, W), F32), pltpu.VMEM((M, W), BF16), pltpu.VMEM((M, Dh), F32),
                pltpu.VMEM((B, D), F32), pltpu.VMEM((4, B, D), F32),
            ],
            compiler_params=pltpu.CompilerParams(vmem_limit_bytes=100 * 1024 * 1024),
            name="adaln_attn_moe_decode",
        )(A_x.reshape(B, D), A_k_cache, A_v_cache, A_wq, A_wo.T, B_w_r, B_w_gate, B_w_up, B_w_down.T, c, w_mod)
        return out.reshape(B, Sq, D)
    return fn


_impl = make(ev=[[(1, 0, 176, 1), (0, 200, 248, 0)], [(0, 192, 8, 1), (0, 1984, 64, 0), (1, 176, 256, 1)], [(0, 456, 248, 0), (0, 448, 8, 1), (1, 432, 256, 1)], [(0, 0, 192, 0), (0, 704, 8, 1), (1, 688, 256, 1)], [(0, 712, 248, 0), (0, 960, 8, 1), (1, 944, 256, 1)], [(0, 968, 248, 0), (0, 1216, 8, 1), (1, 1200, 256, 1)], [(0, 1224, 248, 0), (0, 1472, 8, 1), (1, 1456, 256, 1)], [(0, 1480, 248, 0), (0, 1728, 8, 1), (1, 1712, 248, 1)], [(0, 1736, 248, 0), (1, 1960, 88, 1)]], last=32, wrem=True, split=False, worder='krv')


@jax.jit
def pallas_adaLN_cond__sliding_block_cached__moe_arch_mod__decode_kernel(
    A_x: jax.Array,
    A_k_cache: jax.Array,
    A_v_cache: jax.Array,
    A_wq: jax.Array,
    A_wo: jax.Array,
    B_x: jax.Array,
    B_w_r: jax.Array,
    B_w_gate: jax.Array,
    B_w_up: jax.Array,
    B_w_down: jax.Array,
    c: jax.Array,
    w_mod: jax.Array,
):
    return _impl(A_x, A_k_cache, A_v_cache, A_wq, A_wo, B_x, B_w_r, B_w_gate, B_w_up, B_w_down, c, w_mod)
```

```python
import jax
import jax.numpy as jnp
from jax import lax
import jax.experimental.pallas as pl
import jax.experimental.pallas.tpu as pltpu

F32 = jnp.float32
BF16 = jnp.bfloat16
NT = (((1,), (1,)), ((), ()))

TILE_R, TILE_C = 8, 128
GROUP = 32
LOW_EARLY = 2
REST_AHEAD = 16
HIGH, LOW = 0, 1


def _layernorm(x, eps=1e-05):
    d = x - jnp.mean(x, axis=-1, keepdims=True)
    return d / jnp.sqrt(jnp.mean(d * d, axis=-1, keepdims=True) + eps)


def _sigmoid(x):
    return 1.0 / (1.0 + jnp.exp(-x))


def _cut(lo, hi, phase):
    pts = [lo] + [t for t in range(lo + 1, hi) if (t - phase) % GROUP == 0] + [hi]
    return list(zip(pts[:-1], pts[1:]))


def _rectangles(lo, hi, row_tiles):
    out = []
    while lo < hi:
        r, c = divmod(lo, row_tiles)
        n = min(row_tiles - c, hi - lo)
        out.append((r * TILE_R, c * TILE_C, n * TILE_C))
        lo += n
    return out


def _kv_schedule(window, phase):
    tiles = window // TILE_R
    k = _cut(0, tiles, phase % GROUP)
    v = _cut(0, tiles, (phase - LOW_EARLY) % GROUP)
    assert len(k) == len(v) >= 4
    v[-2:] = [(v[-2][0], v[-1][0] - 1), (v[-1][0] - 1, tiles)]
    rows = lambda which, lo, hi, prio: (which, lo * TILE_R, (hi - lo) * TILE_R, prio)
    high = [rows(0, lo + 1, hi, HIGH) for lo, hi in k[1:-1]]
    high.insert(1, rows(0, *k[-1], HIGH))
    high.insert(3, rows(0, *k[0], HIGH))
    rest = [rows(0, lo, lo + 1, LOW) for lo, _ in k[1:-1]]
    low = [rows(1, lo, hi, LOW) for lo, hi in v]
    groups = [[low[0], high[0]], [rest[0], high[1], low[1]]]
    groups += [[high[i], rest[i - 1], low[i]] for i in range(2, len(k) - 1)]
    return groups + [[high[-1], low[-1]]]


class _Stream:
    def __init__(self, high, low):
        self.high, self.low = high, low
        self.steps = max(len(high), len(low))
        self.step = self.rest = 0

    def advance_to(self, step):
        while self.step < min(step, self.steps):
            if self.step < len(self.high):
                self.high[self.step].start()
            while self.rest < min(self.step + 1 + REST_AHEAD, len(self.high)):
                self.high[self.rest].start_rest()
                self.rest += 1
            if self.step < len(self.low):
                self.low[self.step].start()
            self.step += 1

    def advance(self, steps=1):
        self.advance_to(self.step + steps)

    def start_all_on(self, sem):
        last = max(i for queue in (self.high, self.low) for i, piece in enumerate(queue) if sem in piece.sems)
        self.advance_to(last + 1)


class _Piece:
    def __init__(self, src, dst, sem, sem_of, lo, hi, prio):
        self.src, self.dst, self.sem, self.sem_of, self.prio = src, dst, sem, sem_of, prio
        self.row_tiles = src.shape[1] // TILE_C
        self.lo, self.mid, self.hi = lo, lo + (prio == HIGH), hi
        self.sems = {sem_of(r) for r, _, _ in _rectangles(lo, hi, self.row_tiles)}

    def _start(self, lo, hi, prio):
        for r, c, n in _rectangles(lo, hi, self.row_tiles):
            idx = (pl.ds(r, TILE_R), pl.ds(c, n))
            pltpu.make_async_copy(self.src.at[idx], self.dst.at[idx], self.sem.at[self.sem_of(r)]).start(priority=prio)

    def start(self):
        self._start(self.mid, self.hi, self.prio)

    def start_rest(self):
        self._start(self.lo, self.mid, LOW)


@jax.jit
def pallas_adaLN_cond__sliding_block_cached__moe_arch_mod__decode_kernel(
    A_x: jax.Array,
    A_k_cache: jax.Array,
    A_v_cache: jax.Array,
    A_wq: jax.Array,
    A_wo: jax.Array,
    B_x: jax.Array,
    B_w_r: jax.Array,
    B_w_gate: jax.Array,
    B_w_up: jax.Array,
    B_w_down: jax.Array,
    c: jax.Array,
    w_mod: jax.Array,
):
    del B_x
    B, Sq, D = A_x.shape
    _, Hkv, Sk, Dh = A_k_cache.shape
    Hq = A_wq.shape[1] // Dh
    rep = Hq // Hkv
    F = B_w_gate.shape[1]
    W = min(4096, max(256, Sk // 4))
    assert Sq == 1 and B == TILE_R and D == 576 and Dh == TILE_C
    M = rep * B
    HB = B // 2
    NK, NV = 4, 4
    scale = Dh ** (-0.5)

    ATTN_PHASE, FFN_PHASE = 24, 0
    schedule = _kv_schedule(W, ATTN_PHASE)
    down_parts = [(0, 128), (256, 128), (128, 128), (384, 64), (448, 64), (544, 32), (512, 32)]
    S_SMALL, S_MOD, S_WQ, S_WO, S_WG, S_WU, S_K = range(7)
    S_V = S_K + NK
    S_WD = S_V + NV

    def kernel(x_hbm, k_hbm, v_hbm, wq_hbm, wot_hbm, wr_hbm, wg_hbm, wu_hbm, wdt_hbm, c_hbm, wmod_hbm,
               o_ref,
               x_v, c_v, wr_v, wmod_v, wq_v, wot_v, wg_v, wu_v, wdt_v, kbuf, vbuf,
               q_scr, a_scr, s_scr, p_scr, l_scr, h_scr, mod_scr):

        def body(sem):
            def wait_for(dst, i):
                pltpu.make_async_copy(dst, dst, sem.at[i]).wait()

            def pieces(src, dst, sem_of, phase, prio, lo=0, hi=None):
                hi = src.shape[0] // TILE_R * (src.shape[1] // TILE_C) if hi is None else hi
                phase = phase if prio == HIGH else phase - LOW_EARLY
                return [_Piece(src, dst, sem, sem_of, a, b, prio) for a, b in _cut(lo, hi, phase % GROUP)]

            def k_group(h, b):
                return h % 2 * 2 + b // HB

            def start_kv(h, b, groups):
                for which, row, n, prio in sum(groups, []):
                    src = (k_hbm, v_hbm)[which].at[b, h, pl.ds(Sk - W + row, n)]
                    if which == 0:
                        dst, i = kbuf.at[k_group(h, b), b % HB, pl.ds(row, n)], S_K + k_group(h, b)
                    else:
                        dst, i = vbuf.at[h % NV, b, pl.ds(row, n)], S_V + h % NV
                    pltpu.make_async_copy(src, dst, sem.at[i]).start(priority=prio)

            small = [pltpu.make_async_copy(src, dst, sem.at[S_SMALL])
                     for src, dst in ((c_hbm, c_v), (x_hbm, x_v), (wr_hbm, wr_v))]
            mod_pieces = pieces(wmod_hbm, wmod_v, lambda r: S_MOD, ATTN_PHASE, HIGH)
            wq_pieces = pieces(wq_hbm, wq_v, lambda r: S_WQ, ATTN_PHASE, LOW)
            lead = max(len(wq_pieces) - len(mod_pieces), 0)
            for piece in wq_pieces[:lead]:
                piece.start()
            head = _Stream(mod_pieces, wq_pieces[lead:])
            head.advance_to(head.steps // 3)
            for cp in small:
                cp.start()
            head.advance_to(head.steps)
            s_scr[...] = jnp.zeros_like(s_scr)

            def modulation(i):
                cf = c_v[...].astype(F32)
                m = jnp.dot((cf * _sigmoid(cf)).astype(BF16), wmod_v[:, 2 * i * D:2 * (i + 1) * D],
                            preferred_element_type=F32)
                return m[:, :D], m[:, D:]

            def attn_input():
                for cp in small:
                    cp.wait()
                wait_for(wmod_v, S_MOD)
                sa, ca = modulation(0)
                h_scr[...] = _layernorm(x_v[...].astype(F32)) * (1.0 + ca) + sa

            def keep_modulation(i):
                mod_scr[2 * i], mod_scr[2 * i + 1] = modulation(i + 1)

            def queries(i):
                if i == 0:
                    wait_for(wq_v, S_WQ)
                n = Hkv // 2
                q = jnp.dot(h_scr[...].astype(BF16), wq_v[:, i * n * rep * Dh:(i + 1) * n * rep * Dh],
                            preferred_element_type=F32)
                for t in range(n):
                    heads = [q[:, (rep * t + r) * Dh:(rep * t + r + 1) * Dh] for r in range(rep)]
                    q_scr[i * n + t] = jnp.concatenate(heads, axis=0).astype(BF16)

            def first_step(b, carry):
                start_kv(0, b, schedule)
                work = [attn_input, lambda: keep_modulation(0), lambda: keep_modulation(1),
                        lambda: queries(0), lambda: queries(1)]
                for i, f in enumerate(work):
                    pl.when(b == i + 2)(f)
                return carry

            lax.fori_loop(0, B, first_step, 0)

            row_s = lax.broadcasted_iota(jnp.int32, (M, W), 0) % B
            row_o = lax.broadcasted_iota(jnp.int32, (M, Dh), 0) % B

            def weighted_values(h, b, acc):
                o = jnp.dot(p_scr[...], vbuf[h % NV, b], preferred_element_type=F32)
                return jnp.where(row_o == b, o, acc)

            def phase(h, fetch, values=True, unroll=False):
                if values:
                    wait_for(vbuf.at[(h - 1) % NV], S_V + (h - 1) % NV)

                def step(b, acc):
                    wait_k = lambda: wait_for(kbuf.at[k_group(h, b)], S_K + k_group(h, b))
                    if not unroll:
                        pl.when(b % HB == 0)(wait_k)
                    elif b % HB == 0:
                        wait_k()
                    fetch(b, schedule[:len(schedule) // 2])
                    s = lax.dot_general(q_scr[h], kbuf[k_group(h, b), b % HB], NT, preferred_element_type=F32)
                    s_scr[...] = jnp.where(row_s == b, s, s_scr[...])
                    fetch(b, schedule[len(schedule) // 2:])
                    return weighted_values(h - 1, b, acc) if values else acc

                acc = jnp.zeros((M, Dh), F32)
                if unroll:
                    for b in range(B):
                        acc = step(b, acc)
                else:
                    acc = lax.fori_loop(0, B, step, acc)
                if values:
                    a_scr[h - 1] = acc / l_scr[...]
                s = s_scr[...] * scale
                p = jnp.exp(s - jnp.max(s, axis=-1, keepdims=True))
                l_scr[...] = jnp.broadcast_to(jnp.sum(p, axis=-1, keepdims=True), (M, Dh))
                p_scr[...] = p.astype(BF16)

            def middle_phase(h, carry):
                phase(h, lambda b, groups: start_kv(h + 1, b, groups))
                return carry

            phase(0, lambda b, groups: start_kv(1, b, groups), values=False)
            lax.fori_loop(1, Hkv - 1, middle_phase, 0)

            def down_sem(r):
                return S_WD + [i for i, (lo, n) in enumerate(down_parts) if lo <= r < lo + n][0]

            f_tiles = F // TILE_C
            gate_cut = 36 * GROUP
            down_cut = [row // TILE_R * f_tiles for row in (256, 512, 544, D)]
            down = lambda prio, lo, hi: pieces(wdt_hbm, wdt_v, down_sem, FFN_PHASE, prio, lo, hi)
            tail = _Stream(
                pieces(wu_hbm, wu_v, lambda r: S_WU, FFN_PHASE, HIGH)
                + pieces(wg_hbm, wg_v, lambda r: S_WG, FFN_PHASE, HIGH, hi=gate_cut)
                + down(HIGH, 0, down_cut[0]),
                pieces(wot_hbm, wot_v, lambda r: S_WO, ATTN_PHASE, LOW)
                + pieces(wg_hbm, wg_v, lambda r: S_WG, FFN_PHASE, LOW, lo=gate_cut)
                + down(LOW, down_cut[0], down_cut[1]) + down(LOW, down_cut[2], down_cut[3])
                + down(LOW, down_cut[1], down_cut[2]))

            def arrived(dst, i, step=0):
                tail.advance_to(step)
                tail.start_all_on(i)
                wait_for(dst, i)

            last = Hkv - 1
            phase(last, lambda b, groups: tail.advance(len(groups)), unroll=True)
            wait_for(vbuf.at[last % NV], S_V + last % NV)
            acc = jnp.zeros((M, Dh), F32)
            for b in range(B):
                tail.advance(2)
                acc = weighted_values(last, b, acc)
            a_scr[last] = acc / l_scr[...]

            arrived(wot_v, S_WO, 104)
            proj = None
            for i in range(Hkv // 2):
                heads = [a_scr[t, r * B:(r + 1) * B] for t in (2 * i, 2 * i + 1) for r in range(rep)]
                n = 2 * rep * Dh
                d = lax.dot_general(jnp.concatenate(heads, axis=1).astype(BF16), wot_v[:, i * n:(i + 1) * n],
                                    NT, preferred_element_type=F32)
                proj = d if proj is None else proj + d
                tail.advance(1 + i % 2)
            ga, sb, cb, gb = (mod_scr[i] for i in range(4))
            x1 = x_v[...].astype(F32) + ga * proj
            h2 = _layernorm(x1) * (1.0 + cb) + sb
            h2b = h2.astype(BF16)
            router = jnp.sum(h2b.astype(F32) * wr_v[...].astype(F32).reshape(1, D), axis=-1, keepdims=True)
            route = _sigmoid(router)

            nf = F // 6
            arrived(wu_v, S_WU, 118)
            up = []
            for i in range(F // nf):
                up.append(jnp.dot(h2b, wu_v[:, i * nf:(i + 1) * nf], preferred_element_type=F32))
                tail.advance()
            arrived(wg_v, S_WG, 149)
            act = []
            for i in range(F // nf):
                g = jnp.dot(h2b, wg_v[:, i * nf:(i + 1) * nf], preferred_element_type=F32)
                act.append((g * _sigmoid(g) * up[i]).astype(BF16))
                tail.advance()
            act = jnp.concatenate(act, axis=1)

            y = {}
            for i, (lo, n) in enumerate(down_parts):
                arrived(wdt_v.at[pl.ds(lo, n)], S_WD + i, tail.steps)
                y[lo] = lax.dot_general(act, wdt_v[pl.ds(lo, n)], NT, preferred_element_type=F32)
                start = lo // TILE_C * TILE_C
                cols = slice(start, min(start + TILE_C, D))
                known = [y[t] for t in sorted(y) if cols.start <= t < cols.stop]
                if sum(t.shape[1] for t in known) == cols.stop - cols.start:
                    upd = h2[:, cols] * 0.0 + jnp.concatenate(known, axis=1) * route
                    o_ref[:, cols] = (x1[:, cols] + gb[:, cols] * (h2[:, cols] + upd)).astype(o_ref.dtype)

        pl.run_scoped(body, pltpu.SemaphoreType.DMA((S_WD + len(down_parts),)))

    vmem = pltpu.VMEM
    out = pl.pallas_call(
        kernel,
        out_shape=jax.ShapeDtypeStruct((B, D), A_x.dtype),
        in_specs=[pl.BlockSpec(memory_space=pl.ANY)] * 11,
        out_specs=pl.BlockSpec(memory_space=vmem),
        scratch_shapes=[
            vmem((B, D), A_x.dtype), vmem((B, D), c.dtype), vmem((D,), B_w_r.dtype),
            vmem((D, 6 * D), BF16), vmem((D, Hq * Dh), BF16), vmem((D, Hq * Dh), BF16),
            vmem((D, F), BF16), vmem((D, F), BF16), vmem((D, F), BF16),
            vmem((NK, HB, W, Dh), BF16), vmem((NV, B, W, Dh), BF16),
            vmem((Hkv, M, Dh), BF16), vmem((Hkv, M, Dh), F32),
            vmem((M, W), F32), vmem((M, W), BF16), vmem((M, Dh), F32),
            vmem((B, D), F32), vmem((4, B, D), F32),
        ],
        compiler_params=pltpu.CompilerParams(vmem_limit_bytes=100 * 1024 * 1024),
        name="adaln_attn_moe_decode",
    )(A_x.reshape(B, D), A_k_cache, A_v_cache, A_wq, A_wo.T, B_w_r, B_w_gate, B_w_up, B_w_down.T, c, w_mod)
    return out.reshape(B, Sq, D)
```

```python
import jax
import jax.numpy as jnp
from jax import lax
import jax.experimental.pallas as pl
import jax.experimental.pallas.tpu as pltpu

F32 = jnp.float32
BF16 = jnp.bfloat16
NT = (((1,), (1,)), ((), ()))

TILE_R, TILE_C = 8, 128
GROUP = 32
LOW_EARLY = 2
HIGH, LOW = 0, 1


def _layernorm(x, eps=1e-05):
    d = x - jnp.mean(x, axis=-1, keepdims=True)
    return d / jnp.sqrt(jnp.mean(d * d, axis=-1, keepdims=True) + eps)


def _sigmoid(x):
    return 1.0 / (1.0 + jnp.exp(-x))


def _cut(lo, hi, phase):
    pts = [lo] + [t for t in range(lo + 1, hi) if (t - phase) % GROUP == 0] + [hi]
    return list(zip(pts[:-1], pts[1:]))


def _rectangles(lo, hi, row_tiles):
    out = []
    while lo < hi:
        r, c = divmod(lo, row_tiles)
        n = min(row_tiles - c, hi - lo)
        out.append((r * TILE_R, c * TILE_C, n * TILE_C))
        lo += n
    return out


def _kv_schedule(window, phase):
    tiles = window // TILE_R
    k = _cut(0, tiles, phase % GROUP)
    v = _cut(0, tiles, (phase - LOW_EARLY) % GROUP)
    assert len(k) == len(v) >= 6
    rows = lambda which, lo, hi, prio: (which, lo * TILE_R, (hi - lo) * TILE_R, prio)
    high = [rows(0, lo + 1, hi, HIGH) for lo, hi in k[1:-1]]
    high.insert(1, rows(0, *k[-1], HIGH))
    high.insert(5, rows(0, *k[0], HIGH))
    rest = [rows(0, lo, lo + 1, LOW) for lo, _ in k[1:-1]]
    low = [rows(1, lo, hi, LOW) for lo, hi in v]
    groups = [[low[0], high[0]], [rest[0], high[1], low[1]]]
    groups += [[high[i], rest[i - 1], low[i]] for i in range(2, len(k) - 1)]
    return groups + [[high[-1], low[-1]]]


class _Stream:
    def __init__(self, high, low, ahead):
        self.high, self.low, self.ahead = high, low, ahead
        self.steps = max(len(high), len(low))
        self.step = self.rest = 0

    def advance_to(self, step):
        while self.step < min(step, self.steps):
            if self.step < len(self.high):
                self.high[self.step].start()
            while self.rest < min(self.step + 1 + self.ahead, len(self.high)):
                self.high[self.rest].start_rest()
                self.rest += 1
            if self.step < len(self.low):
                self.low[self.step].start()
            self.step += 1

    def advance(self, steps=1):
        self.advance_to(self.step + steps)

    def start_all_on(self, sem):
        last = max(i for queue in (self.high, self.low) for i, piece in enumerate(queue) if sem in piece.sems)
        self.advance_to(last + 1)


class _Piece:
    def __init__(self, src, dst, sem, sem_of, lo, hi, prio):
        self.src, self.dst, self.sem, self.sem_of, self.prio = src, dst, sem, sem_of, prio
        self.row_tiles = src.shape[1] // TILE_C
        self.lo, self.mid, self.hi = lo, lo + (prio == HIGH), hi
        self.sems = {sem_of(r) for r, _, _ in _rectangles(lo, hi, self.row_tiles)}

    def _start(self, lo, hi, prio):
        for r, c, n in _rectangles(lo, hi, self.row_tiles):
            idx = (pl.ds(r, TILE_R), pl.ds(c, n))
            pltpu.make_async_copy(self.src.at[idx], self.dst.at[idx], self.sem.at[self.sem_of(r)]).start(priority=prio)

    def start(self):
        self._start(self.mid, self.hi, self.prio)

    def start_rest(self):
        self._start(self.lo, self.mid, LOW)


@jax.jit
def pallas_adaLN_cond__sliding_block_cached__moe_arch_mod__decode_kernel(
    A_x: jax.Array,
    A_k_cache: jax.Array,
    A_v_cache: jax.Array,
    A_wq: jax.Array,
    A_wo: jax.Array,
    B_x: jax.Array,
    B_w_r: jax.Array,
    B_w_gate: jax.Array,
    B_w_up: jax.Array,
    B_w_down: jax.Array,
    c: jax.Array,
    w_mod: jax.Array,
):
    del B_x
    B, Sq, D = A_x.shape
    _, Hkv, Sk, Dh = A_k_cache.shape
    Hq = A_wq.shape[1] // Dh
    rep = Hq // Hkv
    F = B_w_gate.shape[1]
    W = min(4096, max(256, Sk // 4))
    assert Sq == 1 and B == TILE_R and D == 576 and Dh == TILE_C
    M = rep * B
    HB = B // 2
    NK, NV = 4, 4
    scale = Dh ** (-0.5)

    ATTN_PHASE, FFN_PHASE = 24, 0
    schedule = _kv_schedule(W, ATTN_PHASE)
    down_parts = [(0, 128), (256, 128), (128, 128), (384, 64), (448, 64), (544, 32), (512, 32)]
    S_SMALL, S_MOD, S_WQ, S_WO, S_WG, S_WU, S_K = range(7)
    S_V = S_K + NK
    S_WD = S_V + NV

    def kernel(x_hbm, k_hbm, v_hbm, wq_hbm, wot_hbm, wr_hbm, wg_hbm, wu_hbm, wdt_hbm, c_hbm, wmod_hbm,
               o_ref,
               x_v, c_v, wr_v, wmod_v, wq_v, wot_v, wg_v, wu_v, wdt_v, kbuf, vbuf,
               q_scr, a_scr, s_scr, p_scr, l_scr, h_scr, mod_scr):

        def body(sem):
            def wait_for(dst, i):
                pltpu.make_async_copy(dst, dst, sem.at[i]).wait()

            def pieces(src, dst, sem_of, phase, prio, lo=0, hi=None):
                hi = src.shape[0] // TILE_R * (src.shape[1] // TILE_C) if hi is None else hi
                phase = phase if prio == HIGH else phase - LOW_EARLY - 1
                return [_Piece(src, dst, sem, sem_of, a, b, prio) for a, b in _cut(lo, hi, phase % GROUP)]

            def k_group(h, b):
                return h % 2 * 2 + b // HB

            def start_kv(h, b, groups):
                for which, row, n, prio in sum(groups, []):
                    src = (k_hbm, v_hbm)[which].at[b, h, pl.ds(Sk - W + row, n)]
                    if which == 0:
                        dst, i = kbuf.at[k_group(h, b), b % HB, pl.ds(row, n)], S_K + k_group(h, b)
                    else:
                        dst, i = vbuf.at[h % NV, b, pl.ds(row, n)], S_V + h % NV
                    pltpu.make_async_copy(src, dst, sem.at[i]).start(priority=prio)

            small = [pltpu.make_async_copy(src, dst, sem.at[S_SMALL])
                     for src, dst in ((c_hbm, c_v), (x_hbm, x_v), (wr_hbm, wr_v))]
            mod_pieces = pieces(wmod_hbm, wmod_v, lambda r: S_MOD, ATTN_PHASE, HIGH)
            wq_pieces = pieces(wq_hbm, wq_v, lambda r: S_WQ, ATTN_PHASE, LOW)
            lead = max(len(wq_pieces) - len(mod_pieces), 0)
            for piece in wq_pieces[:lead]:
                piece.start()
            head = _Stream(mod_pieces, wq_pieces[lead:], ahead=0)
            for cp in small:
                cp.start()
            head.advance_to(head.steps)
            s_scr[...] = jnp.zeros_like(s_scr)

            def modulation(i):
                cf = c_v[...].astype(F32)
                m = jnp.dot((cf * _sigmoid(cf)).astype(BF16), wmod_v[:, 2 * i * D:2 * (i + 1) * D],
                            preferred_element_type=F32)
                return m[:, :D], m[:, D:]

            def attn_input():
                for cp in small:
                    cp.wait()
                wait_for(wmod_v, S_MOD)
                sa, ca = modulation(0)
                h_scr[...] = _layernorm(x_v[...].astype(F32)) * (1.0 + ca) + sa

            def keep_modulation(i):
                mod_scr[2 * i], mod_scr[2 * i + 1] = modulation(i + 1)

            def queries(i):
                if i == 0:
                    wait_for(wq_v, S_WQ)
                n = Hkv // 2
                q = jnp.dot(h_scr[...].astype(BF16), wq_v[:, i * n * rep * Dh:(i + 1) * n * rep * Dh],
                            preferred_element_type=F32)
                for t in range(n):
                    heads = [q[:, (rep * t + r) * Dh:(rep * t + r + 1) * Dh] for r in range(rep)]
                    q_scr[i * n + t] = jnp.concatenate(heads, axis=0).astype(BF16)

            def first_step(b, carry):
                start_kv(0, b, schedule)
                work = [attn_input, lambda: keep_modulation(0), lambda: keep_modulation(1),
                        lambda: queries(0), lambda: queries(1)]
                for i, f in enumerate(work):
                    pl.when(b == i + 2)(f)
                return carry

            lax.fori_loop(0, B, first_step, 0)

            row_s = lax.broadcasted_iota(jnp.int32, (M, W), 0) % B
            row_o = lax.broadcasted_iota(jnp.int32, (M, Dh), 0) % B

            def weighted_values(h, b, acc):
                o = jnp.dot(p_scr[...], vbuf[h % NV, b], preferred_element_type=F32)
                return jnp.where(row_o == b, o, acc)

            def phase(h, fetch, values=True, unroll=False):
                if values:
                    wait_for(vbuf.at[(h - 1) % NV], S_V + (h - 1) % NV)

                def step(b, acc):
                    wait_k = lambda: wait_for(kbuf.at[k_group(h, b)], S_K + k_group(h, b))
                    if not unroll:
                        pl.when(b % HB == 0)(wait_k)
                    elif b % HB == 0:
                        wait_k()
                    fetch(b, schedule[:len(schedule) // 2])
                    s = lax.dot_general(q_scr[h], kbuf[k_group(h, b), b % HB], NT, preferred_element_type=F32)
                    s_scr[...] = jnp.where(row_s == b, s, s_scr[...])
                    fetch(b, schedule[len(schedule) // 2:])
                    return weighted_values(h - 1, b, acc) if values else acc

                acc = jnp.zeros((M, Dh), F32)
                if unroll:
                    for b in range(B):
                        acc = step(b, acc)
                else:
                    acc = lax.fori_loop(0, B, step, acc)
                if values:
                    a_scr[h - 1] = acc / l_scr[...]
                s = s_scr[...] * scale
                p = jnp.exp(s - jnp.max(s, axis=-1, keepdims=True))
                l_scr[...] = jnp.broadcast_to(jnp.sum(p, axis=-1, keepdims=True), (M, Dh))
                p_scr[...] = p.astype(BF16)

            def middle_phase(h, carry):
                phase(h, lambda b, groups: start_kv(h + 1, b, groups))
                return carry

            phase(0, lambda b, groups: start_kv(1, b, groups), values=False)
            lax.fori_loop(1, Hkv - 1, middle_phase, 0)

            def down_sem(r):
                return S_WD + [i for i, (lo, n) in enumerate(down_parts) if lo <= r < lo + n][0]

            f_tiles = F // TILE_C
            gate_cut = 36 * GROUP
            down_cut = [row // TILE_R * f_tiles for row in (256, 512, 544, D)]
            down = lambda prio, lo, hi: pieces(wdt_hbm, wdt_v, down_sem, FFN_PHASE, prio, lo, hi)
            tail = _Stream(
                pieces(wu_hbm, wu_v, lambda r: S_WU, FFN_PHASE, HIGH)
                + pieces(wg_hbm, wg_v, lambda r: S_WG, FFN_PHASE, HIGH, hi=gate_cut)
                + down(HIGH, 0, down_cut[0]),
                pieces(wot_hbm, wot_v, lambda r: S_WO, ATTN_PHASE, LOW)
                + pieces(wg_hbm, wg_v, lambda r: S_WG, FFN_PHASE, LOW, lo=gate_cut)
                + down(LOW, down_cut[0], down_cut[1]) + down(LOW, down_cut[2], down_cut[3])
                + down(LOW, down_cut[1], down_cut[2]),
                ahead=12)

            def arrived(dst, i, step=0):
                tail.advance_to(step)
                tail.start_all_on(i)
                wait_for(dst, i)

            last = Hkv - 1
            phase(last, lambda b, groups: tail.advance(len(groups)), unroll=True)
            wait_for(vbuf.at[last % NV], S_V + last % NV)
            acc = jnp.zeros((M, Dh), F32)
            for b in range(B):
                tail.advance(2)
                acc = weighted_values(last, b, acc)
            a_scr[last] = acc / l_scr[...]

            arrived(wot_v, S_WO, 104)
            proj = None
            for i in range(Hkv // 2):
                heads = [a_scr[t, r * B:(r + 1) * B] for t in (2 * i, 2 * i + 1) for r in range(rep)]
                n = 2 * rep * Dh
                d = lax.dot_general(jnp.concatenate(heads, axis=1).astype(BF16), wot_v[:, i * n:(i + 1) * n],
                                    NT, preferred_element_type=F32)
                proj = d if proj is None else proj + d
                tail.advance(1 + i % 2)
            ga, sb, cb, gb = (mod_scr[i] for i in range(4))
            x1 = x_v[...].astype(F32) + ga * proj
            h2 = _layernorm(x1) * (1.0 + cb) + sb
            h2b = h2.astype(BF16)
            router = jnp.sum(h2b.astype(F32) * wr_v[...].astype(F32).reshape(1, D), axis=-1, keepdims=True)
            route = _sigmoid(router)

            nf = F // 6
            arrived(wu_v, S_WU, 118)
            up = []
            for i in range(F // nf):
                up.append(jnp.dot(h2b, wu_v[:, i * nf:(i + 1) * nf], preferred_element_type=F32))
                tail.advance()
            arrived(wg_v, S_WG, 149)
            act = []
            for i in range(F // nf):
                g = jnp.dot(h2b, wg_v[:, i * nf:(i + 1) * nf], preferred_element_type=F32)
                act.append((g * _sigmoid(g) * up[i]).astype(BF16))
                tail.advance()
            act = jnp.concatenate(act, axis=1)

            y = {}
            for i, (lo, n) in enumerate(down_parts):
                arrived(wdt_v.at[pl.ds(lo, n)], S_WD + i, tail.steps)
                y[lo] = lax.dot_general(act, wdt_v[pl.ds(lo, n)], NT, preferred_element_type=F32)
                start = lo // TILE_C * TILE_C
                cols = slice(start, min(start + TILE_C, D))
                known = [y[t] for t in sorted(y) if cols.start <= t < cols.stop]
                if sum(t.shape[1] for t in known) == cols.stop - cols.start:
                    upd = h2[:, cols] * 0.0 + jnp.concatenate(known, axis=1) * route
                    o_ref[:, cols] = (x1[:, cols] + gb[:, cols] * (h2[:, cols] + upd)).astype(o_ref.dtype)

        pl.run_scoped(body, pltpu.SemaphoreType.DMA((S_WD + len(down_parts),)))

    vmem = pltpu.VMEM
    out = pl.pallas_call(
        kernel,
        out_shape=jax.ShapeDtypeStruct((B, D), A_x.dtype),
        in_specs=[pl.BlockSpec(memory_space=pl.ANY)] * 11,
        out_specs=pl.BlockSpec(memory_space=vmem),
        scratch_shapes=[
            vmem((B, D), A_x.dtype), vmem((B, D), c.dtype), vmem((D,), B_w_r.dtype),
            vmem((D, 6 * D), BF16), vmem((D, Hq * Dh), BF16), vmem((D, Hq * Dh), BF16),
            vmem((D, F), BF16), vmem((D, F), BF16), vmem((D, F), BF16),
            vmem((NK, HB, W, Dh), BF16), vmem((NV, B, W, Dh), BF16),
            vmem((Hkv, M, Dh), BF16), vmem((Hkv, M, Dh), F32),
            vmem((M, W), F32), vmem((M, W), BF16), vmem((M, Dh), F32),
            vmem((B, D), F32), vmem((4, B, D), F32),
        ],
        compiler_params=pltpu.CompilerParams(vmem_limit_bytes=100 * 1024 * 1024),
        name="adaln_attn_moe_decode",
    )(A_x.reshape(B, D), A_k_cache, A_v_cache, A_wq, A_wo.T, B_w_r, B_w_gate, B_w_up, B_w_down.T, c, w_mod)
    return out.reshape(B, Sq, D)
```
